```python
import jax
import jax.numpy as jnp

def _softmax(x, axis=-1):
    return jax.nn.softmax(x, axis=axis)
def _gelu(x):
    return jax.nn.gelu(x, approximate=True)
def _silu(x):
    return jax.nn.silu(x)
def _sigmoid(x):
    return jax.nn.sigmoid(x)
def _layernorm(x, axis=-1, eps=1e-5):
    m = jnp.mean(x, axis=axis, keepdims=True)
    v = jnp.var(x, axis=axis, keepdims=True)
    return (x - m) / jnp.sqrt(v + eps)
def _scatter_add(tgt, idx, src, axis=0):
    return tgt.at[idx].add(src)
def _segment_sum(src, seg, n):
    return jax.ops.segment_sum(src, seg, n)
class _Rng:
    def __init__(self, key):
        self._k = key
    def _next(self):
        self._k, sub = jax.random.split(self._k)
        return sub
    def normal(self, shape):
        return jax.random.normal(self._next(), shape, dtype=jnp.bfloat16)
    def randint(self, lo, hi, shape):
        return jax.random.randint(self._next(), shape, lo, hi, dtype=jnp.int32)
    def uniform(self, shape, lo=0.0, hi=1.0):
        return jax.random.uniform(self._next(), shape, jnp.bfloat16, lo, hi)
    def permutation(self, n):
        return jax.random.permutation(self._next(), n)


kernel_name = 'recurrent_scan__sliding_local_dilated__swiglu_ffn__prompt'

def setup_inputs():
    _rng = _Rng(jax.random.key(int.from_bytes(__import__("os").urandom(4), "little")))
    _w = (lambda a: (lambda t: t.astype(jnp.bfloat16) if jnp.issubdtype(t.dtype, jnp.floating) else t)(jnp.asarray(a)))
    def _A_setup():
        B, S, D = 1, 2048, 1024
        return {
            "x": _w((lambda *s: _rng.normal(s) * 0.05)(B, S, D)),
            "wqkv": _w((lambda *s: _rng.normal(s) * 0.05)(D, 3 * D)),
            "wo": _w((lambda *s: _rng.normal(s) * 0.05)(D, D)),
        }
    _A_in = _A_setup()

    def _B_setup():
        B, S, D, F = 1, 2048, 1024, 3584
        return {
            "x": _w((lambda *s: _rng.normal(s) * 0.05)(B, S, D)),
            "w_gate": _w((lambda *s: _rng.normal(s) * 0.05)(D, F)),
            "w_up": _w((lambda *s: _rng.normal(s) * 0.05)(D, F)),
            "w_down": _w((lambda *s: _rng.normal(s) * 0.05)(F, D)),
        }
    _B_in = _B_setup()

    return {
        "A_x": _A_in["x"],
        "A_wqkv": _A_in["wqkv"],
        "A_wo": _A_in["wo"],
        "B_x": _B_in["x"],
        "B_w_gate": _B_in["w_gate"],
        "B_w_up": _B_in["w_up"],
        "B_w_down": _B_in["w_down"],
    }

def reference(A_x, A_wqkv, A_wo, B_x, B_w_gate, B_w_up, B_w_down):
    def _A_ref(x, wqkv, wo):
        B, S, D = x.shape
        H = 32; Dh = D // H
        W, dil = 8, 2
        qkv = (lambda x, *d: x.transpose(*d))((x @ wqkv).reshape(B, S, 3, H, Dh), 2, 0, 3, 1, 4)
        q, k, v = qkv[0], qkv[1], qkv[2]
        scale = Dh ** -0.5
        pos = jnp.arange(S)
        off = jnp.arange(W) * dil
        idx = pos[:, None] - off[None, :]
        mask = idx >= 0
        idx_c = jnp.where(mask, idx, 0).reshape(-1)
        kg = k[:, :, idx_c, :].reshape(B, H, S, W, Dh)
        vg = v[:, :, idx_c, :].reshape(B, H, S, W, Dh)
        logits = jnp.einsum("bhsd,bhswd->bhsw", q, kg) * scale
        logits = jnp.where(mask[None, None, :, :], logits, -1e9)
        attn = _softmax(logits, axis=-1)
        o = jnp.einsum("bhsw,bhswd->bhsd", attn, vg)
        return (lambda x, *d: x.transpose(*d))(o, 0, 2, 1, 3).reshape(B, S, D) @ wo

    def _B_ref(x, w_gate, w_up, w_down):
        g = _silu(x @ w_gate)
        u = x @ w_up
        return (g * u) @ w_down

    x = A_x
    xn = _layernorm(x, axis=-1)
    s = _A_ref(xn, A_wqkv, A_wo)
    g = _silu(_B_ref(xn, B_w_gate, B_w_up, B_w_down))
    return x + s * g
```

```python
import jax
import jax.numpy as jnp
from jax import lax
from jax.experimental import pallas as pl
from jax.experimental.pallas import tpu as pltpu

S, D, F = 2048, 1024, 3584
H, DH, W, DIL = 32, 32, 8, 2
HALO = 16
LOG2E = 1.4426950408889634
f32, bf16 = jnp.float32, jnp.bfloat16
NN = (((1,), (0,)), ((), ()))
NT = (((1,), (1,)), ((), ()))


def _dot(a, b, dn=NN):
    return lax.dot_general(a, b, dn, preferred_element_type=f32)


def _silu(x):
    e = jnp.exp2(jnp.minimum(x * (-LOG2E), 126.0))
    return x * pltpu.reciprocal(1.0 + e, approx=False, full_range=False)


def make_kernel(bm=256, bg=512, fc=256, tr=16, SCOPES=False, xch=256, nc0=1, dep=True, sched=None):
    nrb = S // bm
    nfc = F // fc
    nxc = S // xch

    def scoped(name, f):
        if SCOPES:
            with jax.named_scope(name):
                f()
        else:
            f()

    def mark(name):
        if SCOPES:
            with jax.named_scope(name):
                pltpu.trace_value(name, jnp.int32(0))

    def ds(i, n):
        return pl.ds(i * n, n) if isinstance(i, int) else pl.ds(pl.multiple_of(i * n, n), n)

    def kernel(x_hbm, wqkv_hbm, wo_hbm, wg_hbm, wu_hbm, wd_hbm, o_hbm,
               x_v, xn_v, wqkv_v, wo_v, wg_v, wu_v, wd_v, wt_v, wop_v,
               h_v, q_s, k_s, v_s, o_s, s_s, f_s, out_v,
               sem_x, sem_g, sem_u, sem_d, sem_a, sem_o):
        def cp_x(r):
            return pltpu.make_async_copy(x_hbm.at[ds(r, xch), :], x_v.at[ds(r, xch), :], sem_x.at[r])
        def cp_g(c):
            return pltpu.make_async_copy(wg_hbm.at[:, ds(c, fc)], wg_v.at[c], sem_g.at[c])
        def cp_u(c):
            return pltpu.make_async_copy(wu_hbm.at[:, ds(c, fc)], wu_v.at[c], sem_u.at[c])
        def cp_d(c):
            return pltpu.make_async_copy(wd_hbm.at[ds(c, fc), :], wd_v.at[c], sem_d.at[c])
        def cp_a(j):
            if j < 3:
                return pltpu.make_async_copy(wqkv_hbm.at[:, pl.ds(j * D, D)], wqkv_v.at[j], sem_a.at[j])
            return pltpu.make_async_copy(wo_hbm, wo_v, sem_a.at[3])
        def cp_o(r, slot):
            return pltpu.make_async_copy(out_v.at[slot], o_hbm.at[ds(r, bm), :], sem_o.at[r])

        def layernorm(xv, xnv, t0, n):
            step = 64
            for t in range(t0, t0 + n, step):
                x = xv[pl.ds(t, step), :].astype(f32)
                m = jnp.mean(x, axis=-1, keepdims=True)
                xc = x - m
                var = jnp.mean(xc * xc, axis=-1, keepdims=True)
                xnv[pl.ds(t, step), :] = (xc * lax.rsqrt(var + 1e-5)).astype(bf16)

        def gate_up(xn, c):
            g = _dot(xn, wg_v[c])
            u = _dot(xn, wu_v[c])
            return (_silu(g) * u).astype(bf16)

        cp_x(0).start()
        for c in range(nc0):
            cp_g(c).start(); cp_u(c).start()
        for c in range(8):
            k_s[c, pl.ds(0, HALO), :] = jnp.zeros((HALO, 128), f32)
            v_s[c, pl.ds(0, HALO), :] = jnp.zeros((HALO, 128), f32)
        scoped('W_x0', lambda: cp_x(0).wait())
        cp_x(1).start()
        layernorm(x_v, xn_v, 0, xch)
        def wait_g0():
            for c in range(nc0):
                cp_g(c).wait(); cp_u(c).wait()
        scoped('W_g0', wait_g0)
        cp_x(2).start()

        def g0_body(r, _):
            @pl.when(r + 3 < nxc)
            def _():
                cp_x(r + 3).start()
            @pl.when(r == nxc - 3)
            def _():
                cp_g(nc0).start(); cp_u(nc0).start()
            @pl.when(r + 1 < nxc)
            def _():
                cp_x(r + 1).wait()
            base = pl.multiple_of(r * xch, xch)
            xv = x_v.at[pl.ds(base, 2 * xch), :]
            xnv = xn_v.at[pl.ds(base, 2 * xch), :]
            xn = xnv[pl.ds(0, xch), :]
            for c in range(nc0):
                h_v[c, ds(r, xch), :] = gate_up(xn, c)
            layernorm(xv, xnv, xch, xch)
            return 0
        mark('M_g0')
        lax.fori_loop(0, nxc, g0_body, 0)
        mark('M_g')

        def g_body(c, _):
            scoped('W_g', lambda: (cp_g(c).wait(), cp_u(c).wait()))
            @pl.when(c + 1 < nfc)
            def _():
                cp_g(c + 1).start(); cp_u(c + 1).start()
            cp_d(c - 1).start()
            for j in range(4):
                @pl.when(c == nc0 + j + 1)
                def _():
                    cp_a(j).start()
            for r0 in range(0, S, bg):
                h_v[c, pl.ds(r0, bg), :] = gate_up(xn_v[pl.ds(r0, bg), :], c)
            return 0
        lax.fori_loop(nc0, nfc, g_body, 0)
        cp_d(nfc - 1).start()
        for c in range(nc0 - 1):
            cp_d(c).start()

        ri = lax.broadcasted_iota(jnp.int32, (128, 128), 0)
        ci = lax.broadcasted_iota(jnp.int32, (128, 128), 1)
        oc, ohl, oj = ri // 16, (ri // 4) % 4, ri % 4
        perm = (ci == ohl * 32 + oc * 4 + oj).astype(bf16)
        def wait_w():
            for j in range(4):
                cp_a(j).wait()
        scoped('W_a', wait_w)
        def perm_body(m, _):
            for i in range(8):
                t = _dot(perm, wqkv_v[m, :, pl.ds(i * 128, 128)], NT).astype(bf16)
                for c in range(8):
                    wt_v[m, pl.ds(c * 128 + 16 * i, 16), :] = t[16 * c:16 * c + 16, :]
            return 0
        lax.fori_loop(0, 3, perm_body, 0)
        for i in range(8):
            t = _dot(perm, wo_v[pl.ds(i * 128, 128), :]).astype(bf16)
            for c in range(8):
                wop_v[pl.ds(c * 128 + 16 * i, 16), :] = t[16 * c:16 * c + 16, :]
        def wait_d():
            for c in range(nfc):
                cp_d(c).wait()
        scoped('W_d', wait_d)
        mark('M_p2')

        qscale = (DH ** -0.5) * LOG2E
        lane = lax.broadcasted_iota(jnp.int32, (tr, 128), 1)
        odd = (lane % 2) == 1
        hi2 = (lane % 4) >= 2

        def fold(x):
            y = x + jnp.where(odd, pltpu.roll(x, 1, 1), pltpu.roll(x, 127, 1))
            return y + jnp.where(hi2, pltpu.roll(y, 2, 1), pltpu.roll(y, 126, 1))

        def qkv(r):
            xn = xn_v[ds(r, bm), :]
            q = _dot(xn, wt_v[0], NT) * qscale
            for c in range(8):
                q_s[c, :, :] = q[:, c * 128:(c + 1) * 128]
            base = pl.multiple_of(r * bm, bm) + HALO
            k = _dot(xn, wt_v[1], NT)
            for c in range(8):
                k_s[c, pl.ds(base, bm), :] = k[:, c * 128:(c + 1) * 128]
            v = _dot(xn, wt_v[2], NT)
            for c in range(8):
                v_s[c, pl.ds(base, bm), :] = v[:, c * 128:(c + 1) * 128]

        def attn_tile(r, kv, vv, t):
            acc = [None] * W
            for c in range(8):
                q = q_s[c, pl.ds(t, tr), :]
                for w in range(W):
                    p = q * kv[c, pl.ds(HALO + t - DIL * w, tr), :]
                    acc[w] = p if acc[w] is None else acc[w] + p
            lg = [fold(a) for a in acc]
            if t < DIL * (W - 1):
                row = lax.broadcasted_iota(jnp.int32, (tr, 128), 0) + (r * bm + t)
                lg = [lg[0]] + [jnp.where(row >= DIL * w, lg[w], -1e9) for w in range(1, W)]
            m = lg[0]
            for w in range(1, W):
                m = jnp.maximum(m, lg[w])
            p = [jnp.exp2(l - m) for l in lg]
            den = p[0]
            for w in range(1, W):
                den = den + p[w]
            rinv = pltpu.reciprocal(den, approx=False, full_range=False)
            for c in range(8):
                o = None
                for w in range(W):
                    tt = p[w] * vv[c, pl.ds(HALO + t - DIL * w, tr), :]
                    o = tt if o is None else o + tt
                o_s[pl.ds(t, tr), pl.ds(c * 128, 128)] = (o * rinv).astype(bf16)

        def fin(r, slot):
            x = x_v[ds(r, bm), :].astype(f32)
            out_v[slot] = (x + s_s[...] * _silu(f_s[...])).astype(bf16)

        ntile = bm // tr
        def p2_body(r, _):
            rb = pl.multiple_of(r * bm, bm)
            kv = k_s.at[:, pl.ds(rb, bm + HALO), :]
            vv = v_s.at[:, pl.ds(rb, bm + HALO), :]
            fin(jnp.maximum(r - 1, 0), r)
            @pl.when(r >= 1)
            def _():
                cp_o(r - 1, r).start()
            qkv(r)
            acc = None
            done = 0
            dummy = jnp.minimum(r + 8, 8)
            for c in range(nfc):
                d = _dot(h_v[c, ds(r, bm), :], wd_v[c])
                if dep:
                    q_s[dummy, 0:8, :] = d[0:8, 0:128]
                tgt = sched[c] if sched else min((ntile * (c + 1) + nfc - 1) // nfc, ntile)
                while done < tgt:
                    attn_tile(r, kv, vv, done * tr); done += 1
                acc = d if acc is None else acc + d
            assert done == ntile
            f_s[...] = acc
            s_s[...] = _dot(o_s[...], wop_v[...])
            mark('M_p2end')
            return 0
        lax.fori_loop(0, nrb, p2_body, 0)
        fin(nrb - 1, nrb)
        cp_o(nrb - 1, nrb).start()
        def wait_o():
            for r in range(nrb):
                cp_o(r, r + 1).wait()
        scoped('W_o', wait_o)

    return kernel


def make_fn(**cfg):
    flags = cfg.pop('flags', None)
    bm = cfg.get('bm', 256); fc = cfg.get('fc', 256); xch = cfg.get('xch', 256)
    kernel = make_kernel(**cfg)
    nrb, nfc = S // bm, F // fc

    def fn(A_x, A_wqkv, A_wo, B_x, B_w_gate, B_w_up, B_w_down):
        x2 = A_x.reshape(S, D)
        anyspec = pl.BlockSpec(memory_space=pl.ANY)
        out = pl.pallas_call(
            kernel,
            out_shape=jax.ShapeDtypeStruct((S, D), bf16),
            in_specs=[anyspec] * 6,
            out_specs=anyspec,
            scratch_shapes=[
                pltpu.VMEM((S + xch, D), bf16),
                pltpu.VMEM((S + xch, D), bf16),
                pltpu.VMEM((3, D, D), bf16),
                pltpu.VMEM((D, D), bf16),
                pltpu.VMEM((nfc, D, fc), bf16),
                pltpu.VMEM((nfc, D, fc), bf16),
                pltpu.VMEM((nfc, fc, D), bf16),
                pltpu.VMEM((3, D, D), bf16),
                pltpu.VMEM((D, D), bf16),
                pltpu.VMEM((nfc, S, fc), bf16),
                pltpu.VMEM((9, bm, 128), f32),
                pltpu.VMEM((8, HALO + S, 128), f32),
                pltpu.VMEM((8, HALO + S, 128), f32),
                pltpu.VMEM((bm, D), bf16),
                pltpu.VMEM((bm, D), f32),
                pltpu.VMEM((bm, D), f32),
                pltpu.VMEM((nrb + 1, bm, D), bf16),
                pltpu.SemaphoreType.DMA((S // xch,)),
                pltpu.SemaphoreType.DMA((nfc,)),
                pltpu.SemaphoreType.DMA((nfc,)),
                pltpu.SemaphoreType.DMA((nfc,)),
                pltpu.SemaphoreType.DMA((4,)),
                pltpu.SemaphoreType.DMA((nrb,)),
            ],
            compiler_params=pltpu.CompilerParams(vmem_limit_bytes=120 * 1024 * 1024, **({'flags': flags} if flags else {})),
        )(x2, A_wqkv, A_wo, B_w_gate, B_w_up, B_w_down)
        return out.reshape(1, S, D)
    return fn


_FN = make_fn(bm=256, bg=512, fc=256)


@jax.jit
def pallas_recurrent_scan__sliding_local_dilated__swiglu_ffn__prompt_kernel(
    A_x, A_wqkv, A_wo, B_x, B_w_gate, B_w_up, B_w_down,
):
    return _FN(A_x, A_wqkv, A_wo, B_x, B_w_gate, B_w_up, B_w_down)
```

```python
import jax
import jax.numpy as jnp
from jax import lax
from jax.experimental import pallas as pl
from jax.experimental.pallas import tpu as pltpu

S, D, F = 2048, 1024, 3584
H, DH, W, DIL = 32, 32, 8, 2
HALO = 16
KPAD = 16
NP = 3 * D // 128
LOG2E = 1.4426950408889634
f32, bf16 = jnp.float32, jnp.bfloat16
NN = (((1,), (0,)), ((), ()))
NT = (((1,), (1,)), ((), ()))


def _dot(a, b, dn=NN):
    return lax.dot_general(a, b, dn, preferred_element_type=f32)


def _silu(x):
    e = jnp.exp2(jnp.minimum(x * (-LOG2E), 126.0))
    return x * pltpu.reciprocal(1.0 + e, approx=False, full_range=False)


def make_kernel(bm=256, bg=512, fc=256, tr=16, SCOPES=False, xch=256, lnstep=16, slots_per=16, slack=10, dfc=512, ngrp=3, lag=1, of32=False, first=0, views=False, kanchor=True, DMARK=False, vanchor=True, rot=True, g0split=(128, 0, 128), gsplit=0, jobskip=1, fin_parts=1, r_wo=5, r_g1=4, xla=1):
    nc0 = 1
    nrb = S // bm
    nfc = F // fc
    nxc = S // xch
    ndc = F // dfc
    gpd = dfc // fc

    def scoped(name, f):
        if SCOPES:
            with jax.named_scope(name):
                f()
        else:
            f()

    def mark(name):
        if SCOPES:
            with jax.named_scope(name):
                pltpu.trace_value(name, jnp.int32(0))

    def ds(i, n):
        return pl.ds(i * n, n) if isinstance(i, int) else pl.ds(pl.multiple_of(i * n, n), n)

    def kernel(x_hbm, wqkv_hbm, wo_hbm, wg_hbm, wu_hbm, wd_hbm, o_hbm,
               x_v, xn_v, wqkv_v, wo_v, wg_v, wu_v, wd_v, wt_v, wop_v,
               h_v, q_s, k_s, v_s, o_s, s_s, f_s, out_v,
               sem_x, sem_g, sem_u, sem_d, sem_a, sem_o):
        def cp_x(r):
            return pltpu.make_async_copy(x_hbm.at[ds(r, xch), :], x_v.at[ds(r, xch), :], sem_x.at[r])
        def cp_g(c):
            return pltpu.make_async_copy(wg_hbm.at[:, ds(c, fc)], wg_v.at[c], sem_g.at[c])
        def cp_u(c):
            return pltpu.make_async_copy(wu_hbm.at[:, ds(c, fc)], wu_v.at[c], sem_u.at[c])
        def cp_d(c):
            return pltpu.make_async_copy(wd_hbm.at[ds(c, fc), :], wd_v.at[c // gpd, ds(c % gpd, fc), :], sem_d.at[c])
        def cp_a(p):
            return pltpu.make_async_copy(wqkv_hbm.at[:, ds(p, 128)], wqkv_v.at[p], sem_a.at[p])
        def cp_wo():
            return pltpu.make_async_copy(wo_hbm, wo_v.at[pl.ds(0, D), :], sem_a.at[NP])
        def cp_o(r, slot):
            return pltpu.make_async_copy(out_v.at[slot], o_hbm.at[ds(r, bm), :], sem_o.at[r])

        def layernorm(xv, xnv, t0, n):
            step = lnstep
            for t in range(t0, t0 + n, step):
                x = xv[pl.ds(t, step), :].astype(f32)
                m = jnp.mean(x, axis=-1, keepdims=True)
                xc = x - m
                var = jnp.mean(xc * xc, axis=-1, keepdims=True)
                xnv[pl.ds(t, step), :] = (xc * lax.rsqrt(var + 1e-5)).astype(bf16)

        def layernorm_dyn(base, n):
            step = lnstep
            for t in range(0, n, step):
                rows = pl.ds(pl.multiple_of(base + t, step), step)
                x = x_v[rows, :].astype(f32)
                m = jnp.mean(x, axis=-1, keepdims=True)
                xc = x - m
                var = jnp.mean(xc * xc, axis=-1, keepdims=True)
                xn_v[rows, :] = (xc * lax.rsqrt(var + 1e-5)).astype(bf16)

        def gate_up(xn, c):
            g = _dot(xn, wg_v[c])
            u = _dot(xn, wu_v[c])
            return (_silu(g) * u).astype(bf16)

        sub_i = lax.broadcasted_iota(jnp.int32, (8, 128), 0)
        lo4 = sub_i < 4
        lo2 = (sub_i % 4) < 2

        def regroup_rows(t):
            tu = pltpu.bitcast(t, jnp.uint32)
            def stage(a, b, sh, m):
                return jnp.where(m, a, pltpu.roll(b, sh, 0)), jnp.where(m, pltpu.roll(a, 8 - sh, 0), b)
            outs = []
            for b in range(2):
                v = [tu[hl * 16 + 8 * b: hl * 16 + 8 * b + 8, :] for hl in range(4)]
                a0, a2 = stage(v[0], v[2], 4, lo4)
                a1, a3 = stage(v[1], v[3], 4, lo4)
                b0, b1 = stage(a0, a1, 2, lo2)
                b2, b3 = stage(a2, a3, 2, lo2)
                outs += [pltpu.bitcast(z, bf16) for z in (b0, b1, b2, b3)]
            return outs

        def permute_strip(p, kt):
            blocks = regroup_rows(wqkv_v[p, pl.ds(kt * 128, 128), :].T)
            m, i = p // 8, p % 8
            for c in range(8):
                o = pl.multiple_of(m * D + c * 128 + 16 * i, 16)
                wt_v[pl.ds(o, 16), pl.ds(kt * 128, 128)] = blocks[c]

        def permute_wo(i, nt):
            blocks = regroup_rows(wo_v[ds(i, 128), pl.ds(nt * 128, 128)])
            for c in range(8):
                o = pl.multiple_of(c * 128 + 16 * i, 16)
                wop_v[pl.ds(o, 16), pl.ds(nt * 128, 128)] = blocks[c]

        cp_x(0).start()
        for c in range(nc0):
            cp_g(c).start(); cp_u(c).start()
        for c in range(8):
            k_s[c, pl.ds(0, HALO), :] = jnp.zeros((HALO, 128), f32)
            v_s[c, pl.ds(0, HALO), :] = jnp.zeros((HALO, 128), f32)
        scoped('W_x0', lambda: cp_x(0).wait())
        cp_x(1).start()
        layernorm(x_v, xn_v, 0, xch)
        def wait_g0():
            for c in range(nc0):
                cp_g(c).wait(); cp_u(c).wait()
        scoped('W_g0', wait_g0)
        for i in range(xla):
            cp_x(2 + i).start()

        def g0_body(r, _):
            @pl.when(r + 2 + xla < nxc)
            def _():
                cp_x(r + 2 + xla).start()
            @pl.when(r == r_wo)
            def _():
                cp_wo().start()
            @pl.when(r == r_g1)
            def _():
                cp_g(nc0).start(); cp_u(nc0).start()
                cp_a(0).start(); cp_a(1).start()
            @pl.when(r + 1 < nxc)
            def _():
                cp_x(r + 1).wait()
            if g0split:
                nt = fc // 128
                pa, pb, pc_ = g0split
                assert pa + pb + pc_ == xch and nt == 2
                nb = (r + 1) * xch
                xl = lambda: xn_v[ds(r, xch), :]
                g = _dot(xl(), wg_v[0, :, pl.ds(0, 128)])
                u = _dot(xl(), wu_v[0, :, pl.ds(0, 128)])
                h_v[0, ds(r, xch), pl.ds(0, 128)] = (_silu(g) * u).astype(bf16)
                if pa: layernorm_dyn(nb, pa)
                g = _dot(xl(), wg_v[0, :, pl.ds(128, 128)])
                if pb: layernorm_dyn(nb + pa, pb)
                u = _dot(xl(), wu_v[0, :, pl.ds(128, 128)])
                h_v[0, ds(r, xch), pl.ds(128, 128)] = (_silu(g) * u).astype(bf16)
                if pc_: layernorm_dyn(nb + pa + pb, pc_)
            else:
                base = pl.multiple_of(r * xch, xch)
                xv = x_v.at[pl.ds(base, 2 * xch), :]
                xnv = xn_v.at[pl.ds(base, 2 * xch), :]
                xn = xnv[pl.ds(0, xch), :]
                h_v[0, ds(r, xch), pl.ds(0, fc)] = gate_up(xn, 0)
                layernorm(xv, xnv, xch, xch)
            return 0
        mark('M_g0')
        lax.fori_loop(0, nxc, g0_body, 0)
        mark('M_g')

        def g_body(c, _):
            j = c - nc0
            p0 = jnp.maximum(2 * j - 2, 0)
            scoped('W_g', lambda: (cp_g(c).wait(), cp_u(c).wait()))
            def wait_a():
                @pl.when(j == 0)
                def _():
                    cp_wo().wait()
                @pl.when(j != 1)
                def _():
                    cp_a(p0).wait(); cp_a(p0 + 1).wait()
            scoped('W_a', wait_a)
            @pl.when(c + 1 < nfc)
            def _():
                cp_g(c + 1).start(); cp_u(c + 1).start()
            @pl.when(jnp.logical_and(j >= 1, 2 * j < NP))
            def _():
                cp_a(2 * j).start(); cp_a(2 * j + 1).start()
            @pl.when(c + 1 < nfc)
            def _():
                cp_d(c).start()
            @pl.when(c == nc0)
            def _():
                cp_d(0).start(); cp_d(nfc - 1).start()
            jobs = []
            for kt in range(8):
                jobs += [('a', 0, kt), ('a', 1, kt), ('o', 0, kt)]
            nblk = S // bg
            nb_use = nblk - jobskip
            cuts = [len(jobs) * i // nb_use for i in range(nb_use + 1)] + [len(jobs)] * jobskip
            da = jnp.minimum(c + NP, NP)
            do = pl.multiple_of(jnp.minimum(c + 64, 64) * 16, 16)
            for ib, r0 in enumerate(range(0, S, bg)):
                if gsplit == 1 or (gsplit == 2 and ib == nblk - 1):
                    hs = []
                    for jj in range(fc // 128):
                        g = _dot(xn_v[pl.ds(r0, bg), :], wg_v[c, :, pl.ds(jj * 128, 128)])
                        u = _dot(xn_v[pl.ds(r0, bg), :], wu_v[c, :, pl.ds(jj * 128, 128)])
                        hs.append((_silu(g) * u).astype(bf16))
                        h_v[c // gpd, pl.ds(r0, bg), ds((c % gpd) * (fc // 128) + jj, 128)] = hs[-1]
                    hh = jnp.concatenate(hs, axis=1)
                else:
                    hh = gate_up(xn_v[pl.ds(r0, bg), :], c)
                    h_v[c // gpd, pl.ds(r0, bg), ds(c % gpd, fc)] = hh
                per = cuts[ib + 1] - cuts[ib]
                for u in range(per):
                    kind, dp, kt = jobs[cuts[ib] + u]
                    ar = (u * bg // per) // 16 * 16
                    anchor = hh[ar:ar + 16, 0:128]
                    if kind == 'a':
                        wqkv_v[da, 0:16, :] = anchor
                        permute_strip(p0 + dp, kt)
                    else:
                        wo_v[pl.ds(do, 16), 0:128] = anchor
                        permute_wo(jnp.minimum(j, 7), kt)
            return 0
        assert 2 * (nfc - nc0 - 1) >= NP and nfc - nc0 >= 8
        lax.fori_loop(nc0, nfc, g_body, 0)
        def wait_d():
            for c in range(nfc):
                cp_d(c).wait()
        scoped('W_d', wait_d)
        mark('M_p2')

        qscale = (DH ** -0.5) * LOG2E
        lane = lax.broadcasted_iota(jnp.int32, (tr, 128), 1)
        odd = (lane % 2) == 1
        hi2 = (lane % 4) >= 2

        def fold(x):
            y = x + jnp.where(odd, pltpu.roll(x, 1, 1), pltpu.roll(x, 127, 1))
            return y + jnp.where(hi2, pltpu.roll(y, 2, 1), pltpu.roll(y, 126, 1))

        def qkv(r):
            xn = xn_v[ds(r, bm), :]
            q = _dot(xn, wt_v[pl.ds(0, D), :], NT) * qscale
            for c in range(8):
                q_s[c, :, :] = q[:, c * 128:(c + 1) * 128]
            base = pl.multiple_of(r * bm, bm) + HALO
            k = _dot(xn, wt_v[pl.ds(D, D), :], NT)
            for c in range(8):
                k_s[c, pl.ds(base, bm), :] = k[:, c * 128:(c + 1) * 128]
            v = _dot(xn, wt_v[pl.ds(2 * D, D), :], NT)
            for c in range(8):
                v_s[c, pl.ds(base, bm), :] = v[:, c * 128:(c + 1) * 128]

        groups = {1: [tuple(range(8))], 2: [(0, 1, 2, 3), (4, 5, 6, 7)], 3: [(0, 1, 2), (3, 4, 5), (6, 7)], 4: [(0, 1), (2, 3), (4, 5), (6, 7)]}[ngrp]

        def attn_qk(rb, t, g, st):
            acc = st.setdefault('acc', [None] * W)
            for c in groups[g]:
                q = q_s[c, pl.ds(t, tr), :]
                for w in range(W):
                    p = q * (rb[0][c, pl.ds(HALO + t - DIL * w, tr), :] if views else k_s[c, pl.ds(rb + (HALO + t - DIL * w), tr), :])
                    acc[w] = p if acc[w] is None else acc[w] + p

        def attn_softmax(r, t, st):
            lg = [fold(a) for a in st.pop('acc')]
            if t < DIL * (W - 1):
                row = lax.broadcasted_iota(jnp.int32, (tr, 128), 0) + (r * bm + t)
                lg = [lg[0]] + [jnp.where(row >= DIL * w, lg[w], -1e9) for w in range(1, W)]
            m = lg[0]
            for w in range(1, W):
                m = jnp.maximum(m, lg[w])
            p = [jnp.exp2(l - m) for l in lg]
            den = p[0]
            for w in range(1, W):
                den = den + p[w]
            st['p'] = p
            st['rinv'] = pltpu.reciprocal(den, approx=False, full_range=False)

        def attn_pv(rb, t, g, st):
            p = st['p']
            for c in groups[g]:
                o = None
                for w in range(W):
                    tt = p[w] * (rb[1][c, pl.ds(HALO + t - DIL * w, tr), :] if views else v_s[c, pl.ds(rb + (HALO + t - DIL * w), tr), :])
                    o = tt if o is None else o + tt
                o_s[pl.ds(t, tr), pl.ds(c * 128, 128)] = (o * st['rinv']).astype(f32 if of32 else bf16)

        def fin(r, slot):
            x = x_v[ds(r, bm), :].astype(f32)
            out_v[slot] = (x + s_s[...] * _silu(f_s[...])).astype(bf16)

        ntile = bm // tr
        def p2_body(r, _):
            rb = pl.multiple_of(r * bm, bm)
            fin(jnp.maximum(r - 1, 0), r)
            @pl.when(r >= 1)
            def _():
                cp_o(r - 1, r).start()
            qkv(r)
            if views:
                rb = (k_s.at[:, pl.ds(rb, bm + HALO), :], v_s.at[:, pl.ds(rb, bm + HALO), :])
            items = []
            for t in range(ntile + lag):
                if t < ntile:
                    items += [('qk', t, g) for g in range(ngrp)]
                if t >= lag:
                    items += [('pv', t - lag, g) for g in range(ngrp)]
            nslot = ndc * slots_per
            span = nslot - slack - first
            by_slot = {}
            for i, it in enumerate(items):
                by_slot.setdefault(first + i * span // len(items), []).append(it)
            sts = [dict() for _ in range(ntile)]
            dummy = jnp.minimum(r + 8, 8)
            dummy2 = jnp.minimum(r, 7)
            acc = None
            for c in range(ndc):
                if DMARK: mark('D%d' % c)
                d = _dot(h_v[c, ds(r, bm), :], wd_v[c])
                npass = 8 * 512 // dfc if dfc >= 512 else 4
                per_pass = slots_per // npass
                for u in range(slots_per):
                    todo = by_slot.get(c * slots_per + u, [])
                    if not todo:
                        continue
                    pp, hf = u // per_pass, u % per_pass
                    col = pp * (1024 // npass)
                    anchor = d[hf * (bm // per_pass): hf * (bm // per_pass) + 8, col:col + 128]
                    kinds = set(k for k, _, _ in todo)
                    ro = 8 * ((c * slots_per + u) % 32) if rot else 0
                    if 'qk' in kinds:
                        q_s[dummy, ro:ro + 8, :] = anchor
                        if kanchor:
                            k_s[dummy2, HALO + S:HALO + S + 8, :] = anchor
                    if 'pv' in kinds:
                        if vanchor:
                            v_s[dummy2, HALO + S:HALO + S + 8, :] = anchor
                    for kind, t, g in todo:
                        if kind == 'qk':
                            attn_qk(rb, t * tr, g, sts[t])
                            if g == ngrp - 1:
                                attn_softmax(r, t * tr, sts[t])
                        else:
                            attn_pv(rb, t * tr, g, sts[t])
                acc = d if acc is None else acc + d
            f_s[...] = acc
            if DMARK: mark('Dend')
            s_s[...] = _dot(o_s[...].astype(bf16), wop_v[...])
            mark('M_p2end')
            return 0
        lax.fori_loop(0, nrb, p2_body, 0)
        npo = fin_parts
        pr = bm // npo
        def cp_last(i):
            return pltpu.make_async_copy(out_v.at[nrb, pl.ds(i * pr, pr), :],
                                         o_hbm.at[pl.ds((nrb - 1) * bm + i * pr, pr), :], sem_o.at[nrb - 1])
        for i in range(npo):
            rows = pl.ds(i * pr, pr)
            x = x_v[pl.ds((nrb - 1) * bm + i * pr, pr), :].astype(f32)
            out_v[nrb, rows, :] = (x + s_s[rows, :] * _silu(f_s[rows, :])).astype(bf16)
            cp_last(i).start()
        def wait_o():
            for r in range(nrb - 1):
                cp_o(r, r + 1).wait()
            for i in range(npo):
                cp_last(i).wait()
        scoped('W_o', wait_o)

    return kernel


def make_fn(**cfg):
    flags = cfg.pop('flags', None)
    bm = cfg.get('bm', 256); fc = cfg.get('fc', 256); xch = cfg.get('xch', 256)
    kernel = make_kernel(**cfg)
    nrb, nfc = S // bm, F // fc
    dfc = cfg.get('dfc', 512)

    def fn(A_x, A_wqkv, A_wo, B_x, B_w_gate, B_w_up, B_w_down):
        x2 = A_x.reshape(S, D)
        anyspec = pl.BlockSpec(memory_space=pl.ANY)
        out = pl.pallas_call(
            kernel,
            out_shape=jax.ShapeDtypeStruct((S, D), bf16),
            in_specs=[anyspec] * 6,
            out_specs=anyspec,
            scratch_shapes=[
                pltpu.VMEM((S + xch, D), bf16),
                pltpu.VMEM((S + xch, D), bf16),
                pltpu.VMEM((NP + 1, D, 128), bf16),
                pltpu.VMEM((D + 64, D), bf16),
                pltpu.VMEM((nfc, D, fc), bf16),
                pltpu.VMEM((nfc, D, fc), bf16),
                pltpu.VMEM((F // dfc, dfc, D), bf16),
                pltpu.VMEM((3 * D, D), bf16),
                pltpu.VMEM((D, D), bf16),
                pltpu.VMEM((F // dfc, S, dfc), bf16),
                pltpu.VMEM((9, bm, 128), f32),
                pltpu.VMEM((8, HALO + S + KPAD, 128), f32),
                pltpu.VMEM((8, HALO + S + KPAD, 128), f32),
                pltpu.VMEM((bm, D), f32 if cfg.get('of32', False) else bf16),
                pltpu.VMEM((bm, D), f32),
                pltpu.VMEM((bm, D), f32),
                pltpu.VMEM((nrb + 1, bm, D), bf16),
                pltpu.SemaphoreType.DMA((S // xch,)),
                pltpu.SemaphoreType.DMA((nfc,)),
                pltpu.SemaphoreType.DMA((nfc,)),
                pltpu.SemaphoreType.DMA((nfc,)),
                pltpu.SemaphoreType.DMA((NP + 1,)),
                pltpu.SemaphoreType.DMA((nrb,)),
            ],
            compiler_params=pltpu.CompilerParams(vmem_limit_bytes=120 * 1024 * 1024, disable_bounds_checks=True, disable_semaphore_checks=True, **({'flags': flags} if flags else {})),
        )(x2, A_wqkv, A_wo, B_w_gate, B_w_up, B_w_down)
        return out.reshape(1, S, D)
    return fn


_FN = make_fn(bm=256, bg=512, fc=256, ngrp=2, slack=27, xla=1, r_wo=5, r_g1=4)


@jax.jit
def pallas_recurrent_scan__sliding_local_dilated__swiglu_ffn__prompt_kernel(
    A_x, A_wqkv, A_wo, B_x, B_w_gate, B_w_up, B_w_down,
):
    return _FN(A_x, A_wqkv, A_wo, B_x, B_w_gate, B_w_up, B_w_down)
```

```python
import jax
import jax.numpy as jnp
from jax import lax
from jax.experimental import pallas as pl
from jax.experimental.pallas import tpu as pltpu

S, D, F = 2048, 1024, 3584
H, DH, W, DIL = 32, 32, 8, 2
HALO = 16
KPAD = 16
NP = 3 * D // 128
LOG2E = 1.4426950408889634
f32, bf16 = jnp.float32, jnp.bfloat16
NN = (((1,), (0,)), ((), ()))
NT = (((1,), (1,)), ((), ()))


def _dot(a, b, dn=NN):
    return lax.dot_general(a, b, dn, preferred_element_type=f32)


def _silu(x):
    e = jnp.exp2(jnp.minimum(x * (-LOG2E), 126.0))
    return x * pltpu.reciprocal(1.0 + e, approx=False, full_range=False)


def make_kernel(bm=256, bg=512, fc=256, tr=16, SCOPES=False, xch=256, lnstep=16, slots_per=16, slack=10, dfc=512, ngrp=3, lag=1, of32=False, first=0, views=False, kanchor=True, DMARK=False, vanchor=True, rot=True, g0split=(128, 0, 128), gsplit=0, jobskip=1, fin_inline=1, peel=1, lnmid=0, r_wo=5, r_g1=4, xla=1):
    nc0 = 1
    nrb = S // bm
    nfc = F // fc
    nxc = S // xch
    ndc = F // dfc
    gpd = dfc // fc

    def scoped(name, f):
        if SCOPES:
            with jax.named_scope(name):
                f()
        else:
            f()

    def mark(name):
        if SCOPES:
            with jax.named_scope(name):
                pltpu.trace_value(name, jnp.int32(0))

    def ds(i, n):
        return pl.ds(i * n, n) if isinstance(i, int) else pl.ds(pl.multiple_of(i * n, n), n)

    def kernel(x_hbm, wqkv_hbm, wo_hbm, wg_hbm, wu_hbm, wd_hbm, o_hbm,
               x_v, xn_v, wqkv_v, wo_v, wg_v, wu_v, wd_v, wt_v, wop_v,
               h_v, q_s, k_s, v_s, o_s, s_s, f_s, out_v,
               sem_x, sem_g, sem_u, sem_d, sem_a, sem_o, sem_p):
        def cp_x(r):
            return pltpu.make_async_copy(x_hbm.at[ds(r, xch), :], x_v.at[ds(r, xch), :], sem_x.at[r])
        def cp_g(c):
            return pltpu.make_async_copy(wg_hbm.at[:, ds(c, fc)], wg_v.at[c], sem_g.at[c])
        def cp_u(c):
            return pltpu.make_async_copy(wu_hbm.at[:, ds(c, fc)], wu_v.at[c], sem_u.at[c])
        def cp_d(c):
            return pltpu.make_async_copy(wd_hbm.at[ds(c, fc), :], wd_v.at[c // gpd, ds(c % gpd, fc), :], sem_d.at[c])
        def cp_a(p):
            return pltpu.make_async_copy(wqkv_hbm.at[:, ds(p, 128)], wqkv_v.at[p], sem_a.at[p])
        def cp_wo():
            return pltpu.make_async_copy(wo_hbm, wo_v.at[pl.ds(0, D), :], sem_a.at[NP])
        def cp_o(r, slot):
            return pltpu.make_async_copy(out_v.at[slot], o_hbm.at[ds(r, bm), :], sem_o.at[r])

        def layernorm(xv, xnv, t0, n):
            step = lnstep
            for t in range(t0, t0 + n, step):
                x = xv[pl.ds(t, step), :].astype(f32)
                m = jnp.mean(x, axis=-1, keepdims=True)
                xc = x - m
                var = jnp.mean(xc * xc, axis=-1, keepdims=True)
                xnv[pl.ds(t, step), :] = (xc * lax.rsqrt(var + 1e-5)).astype(bf16)

        def layernorm_dyn(base, n):
            step = lnstep
            for t in range(0, n, step):
                rows = pl.ds(pl.multiple_of(base + t, step), step)
                x = x_v[rows, :].astype(f32)
                m = jnp.mean(x, axis=-1, keepdims=True)
                xc = x - m
                var = jnp.mean(xc * xc, axis=-1, keepdims=True)
                xn_v[rows, :] = (xc * lax.rsqrt(var + 1e-5)).astype(bf16)

        def gate_up(xn, c):
            g = _dot(xn, wg_v[c])
            u = _dot(xn, wu_v[c])
            return (_silu(g) * u).astype(bf16)

        sub_i = lax.broadcasted_iota(jnp.int32, (8, 128), 0)
        lo4 = sub_i < 4
        lo2 = (sub_i % 4) < 2

        def regroup_rows(t):
            tu = pltpu.bitcast(t, jnp.uint32)
            def stage(a, b, sh, m):
                return jnp.where(m, a, pltpu.roll(b, sh, 0)), jnp.where(m, pltpu.roll(a, 8 - sh, 0), b)
            outs = []
            for b in range(2):
                v = [tu[hl * 16 + 8 * b: hl * 16 + 8 * b + 8, :] for hl in range(4)]
                a0, a2 = stage(v[0], v[2], 4, lo4)
                a1, a3 = stage(v[1], v[3], 4, lo4)
                b0, b1 = stage(a0, a1, 2, lo2)
                b2, b3 = stage(a2, a3, 2, lo2)
                outs += [pltpu.bitcast(z, bf16) for z in (b0, b1, b2, b3)]
            return outs

        def permute_strip(p, kt):
            blocks = regroup_rows(wqkv_v[p, pl.ds(kt * 128, 128), :].T)
            m, i = p // 8, p % 8
            for c in range(8):
                o = pl.multiple_of(m * D + c * 128 + 16 * i, 16)
                wt_v[pl.ds(o, 16), pl.ds(kt * 128, 128)] = blocks[c]

        def permute_wo(i, nt):
            blocks = regroup_rows(wo_v[ds(i, 128), pl.ds(nt * 128, 128)])
            for c in range(8):
                o = pl.multiple_of(c * 128 + 16 * i, 16)
                wop_v[pl.ds(o, 16), pl.ds(nt * 128, 128)] = blocks[c]

        def cp_p(i):
            src, dst = (wg_hbm, wg_v) if i % 2 == 0 else (wu_hbm, wu_v)
            cols = pl.ds((i // 2) * 128, 128)
            return pltpu.make_async_copy(src.at[:, cols], dst.at[0, :, cols], sem_p.at[i])
        for c in range(8):
            k_s[c, pl.ds(0, HALO), :] = jnp.zeros((HALO, 128), f32)
            v_s[c, pl.ds(0, HALO), :] = jnp.zeros((HALO, 128), f32)
        if peel >= 3:
            cp_x(0).start(); cp_p(0).start(); cp_p(1).start()
            scoped('W_x0', lambda: cp_x(0).wait())
            cp_p(2).start(); cp_p(3).start()
            if peel == 3:
                cp_x(1).start()
            layernorm(x_v, xn_v, 0, xch)
            xl = lambda: xn_v[pl.ds(0, xch), :]
            scoped('W_a0', lambda: (cp_p(0).wait(), cp_p(1).wait()))
            if peel == 4:
                cp_x(1).start()
            g = _dot(xl(), wg_v[0, :, pl.ds(0, 128)])
            u = _dot(xl(), wu_v[0, :, pl.ds(0, 128)])
            h_v[0, pl.ds(0, xch), pl.ds(0, 128)] = (_silu(g) * u).astype(bf16)
            scoped('W_b0', lambda: (cp_p(2).wait(), cp_p(3).wait()))
            scoped('W_x1', lambda: cp_x(1).wait())
            for i in range(0, xla + 1):
                cp_x(2 + i).start()
            g = _dot(xl(), wg_v[0, :, pl.ds(128, 128)])
            if lnmid:
                layernorm(x_v, xn_v, xch, lnmid)
            u = _dot(xl(), wu_v[0, :, pl.ds(128, 128)])
            h_v[0, pl.ds(0, xch), pl.ds(128, 128)] = (_silu(g) * u).astype(bf16)
            layernorm(x_v, xn_v, xch + lnmid, xch - lnmid)
        elif peel:
            assert fc == 256
            cp_x(0).start(); cp_p(0).start(); cp_p(1).start()
            scoped('W_x0', lambda: cp_x(0).wait())
            cp_p(2).start()
            if peel == 1:
                cp_p(3).start()
            layernorm(x_v, xn_v, 0, xch)
            xl = lambda: xn_v[pl.ds(0, xch), :]
            scoped('W_ga', lambda: cp_p(0).wait())
            if peel == 2:
                cp_x(1).start()
            g = _dot(xl(), wg_v[0, :, pl.ds(0, 128)])
            scoped('W_ua', lambda: cp_p(1).wait())
            if peel == 1:
                cp_x(1).start()
            else:
                cp_p(3).start()
            u = _dot(xl(), wu_v[0, :, pl.ds(0, 128)])
            h_v[0, pl.ds(0, xch), pl.ds(0, 128)] = (_silu(g) * u).astype(bf16)
            scoped('W_gb', lambda: cp_p(2).wait())
            cp_x(2).start()
            g = _dot(xl(), wg_v[0, :, pl.ds(128, 128)])
            if peel == 2:
                scoped('W_x1', lambda: cp_x(1).wait())
            scoped('W_ub', lambda: cp_p(3).wait())
            u = _dot(xl(), wu_v[0, :, pl.ds(128, 128)])
            h_v[0, pl.ds(0, xch), pl.ds(128, 128)] = (_silu(g) * u).astype(bf16)
            if peel == 2:
                layernorm(x_v, xn_v, xch, xch)
            if peel == 1:
                scoped('W_x1', lambda: cp_x(1).wait())
                layernorm(x_v, xn_v, xch, xch)
            for i in range(1, xla + 1):
                cp_x(2 + i).start()
        else:
            cp_x(0).start()
            for c in range(nc0):
                cp_g(c).start(); cp_u(c).start()
            scoped('W_x0', lambda: cp_x(0).wait())
            cp_x(1).start()
            layernorm(x_v, xn_v, 0, xch)
            def wait_g0():
                for c in range(nc0):
                    cp_g(c).wait(); cp_u(c).wait()
            scoped('W_g0', wait_g0)
            for i in range(xla):
                cp_x(2 + i).start()

        def g0_body(r, _):
            @pl.when(r + 2 + xla < nxc)
            def _():
                cp_x(r + 2 + xla).start()
            @pl.when(r == r_wo)
            def _():
                cp_wo().start()
            @pl.when(r == r_g1)
            def _():
                cp_g(nc0).start(); cp_u(nc0).start()
                cp_a(0).start(); cp_a(1).start()
            @pl.when(r + 1 < nxc)
            def _():
                cp_x(r + 1).wait()
            if g0split:
                nt = fc // 128
                pa, pb, pc_ = g0split
                assert pa + pb + pc_ == xch and nt == 2
                nb = (r + 1) * xch
                xl = lambda: xn_v[ds(r, xch), :]
                g = _dot(xl(), wg_v[0, :, pl.ds(0, 128)])
                u = _dot(xl(), wu_v[0, :, pl.ds(0, 128)])
                h_v[0, ds(r, xch), pl.ds(0, 128)] = (_silu(g) * u).astype(bf16)
                if pa: layernorm_dyn(nb, pa)
                g = _dot(xl(), wg_v[0, :, pl.ds(128, 128)])
                if pb: layernorm_dyn(nb + pa, pb)
                u = _dot(xl(), wu_v[0, :, pl.ds(128, 128)])
                h_v[0, ds(r, xch), pl.ds(128, 128)] = (_silu(g) * u).astype(bf16)
                if pc_: layernorm_dyn(nb + pa + pb, pc_)
            else:
                base = pl.multiple_of(r * xch, xch)
                xv = x_v.at[pl.ds(base, 2 * xch), :]
                xnv = xn_v.at[pl.ds(base, 2 * xch), :]
                xn = xnv[pl.ds(0, xch), :]
                h_v[0, ds(r, xch), pl.ds(0, fc)] = gate_up(xn, 0)
                layernorm(xv, xnv, xch, xch)
            return 0
        mark('M_g0')
        lax.fori_loop(1 if peel else 0, nxc, g0_body, 0)
        mark('M_g')

        def g_body(c, _):
            j = c - nc0
            p0 = jnp.maximum(2 * j - 2, 0)
            scoped('W_g', lambda: (cp_g(c).wait(), cp_u(c).wait()))
            def wait_a():
                @pl.when(j == 0)
                def _():
                    cp_wo().wait()
                @pl.when(j != 1)
                def _():
                    cp_a(p0).wait(); cp_a(p0 + 1).wait()
            scoped('W_a', wait_a)
            @pl.when(c + 1 < nfc)
            def _():
                cp_g(c + 1).start(); cp_u(c + 1).start()
            @pl.when(jnp.logical_and(j >= 1, 2 * j < NP))
            def _():
                cp_a(2 * j).start(); cp_a(2 * j + 1).start()
            @pl.when(c + 1 < nfc)
            def _():
                cp_d(c).start()
            @pl.when(c == nc0)
            def _():
                cp_d(0).start(); cp_d(nfc - 1).start()
            jobs = []
            for kt in range(8):
                jobs += [('a', 0, kt), ('a', 1, kt), ('o', 0, kt)]
            nblk = S // bg
            nb_use = nblk - jobskip
            cuts = [len(jobs) * i // nb_use for i in range(nb_use + 1)] + [len(jobs)] * jobskip
            da = jnp.minimum(c + NP, NP)
            do = pl.multiple_of(jnp.minimum(c + 64, 64) * 16, 16)
            for ib, r0 in enumerate(range(0, S, bg)):
                if gsplit == 1 or (gsplit == 2 and ib == nblk - 1):
                    hs = []
                    for jj in range(fc // 128):
                        g = _dot(xn_v[pl.ds(r0, bg), :], wg_v[c, :, pl.ds(jj * 128, 128)])
                        u = _dot(xn_v[pl.ds(r0, bg), :], wu_v[c, :, pl.ds(jj * 128, 128)])
                        hs.append((_silu(g) * u).astype(bf16))
                        h_v[c // gpd, pl.ds(r0, bg), ds((c % gpd) * (fc // 128) + jj, 128)] = hs[-1]
                    hh = jnp.concatenate(hs, axis=1)
                else:
                    hh = gate_up(xn_v[pl.ds(r0, bg), :], c)
                    h_v[c // gpd, pl.ds(r0, bg), ds(c % gpd, fc)] = hh
                per = cuts[ib + 1] - cuts[ib]
                for u in range(per):
                    kind, dp, kt = jobs[cuts[ib] + u]
                    ar = (u * bg // per) // 16 * 16
                    anchor = hh[ar:ar + 16, 0:128]
                    if kind == 'a':
                        wqkv_v[da, 0:16, :] = anchor
                        permute_strip(p0 + dp, kt)
                    else:
                        wo_v[pl.ds(do, 16), 0:128] = anchor
                        permute_wo(jnp.minimum(j, 7), kt)
            return 0
        assert 2 * (nfc - nc0 - 1) >= NP and nfc - nc0 >= 8
        lax.fori_loop(nc0, nfc, g_body, 0)
        def wait_d():
            for c in range(nfc):
                cp_d(c).wait()
        scoped('W_d', wait_d)
        mark('M_p2')

        qscale = (DH ** -0.5) * LOG2E
        lane = lax.broadcasted_iota(jnp.int32, (tr, 128), 1)
        odd = (lane % 2) == 1
        hi2 = (lane % 4) >= 2

        def fold(x):
            y = x + jnp.where(odd, pltpu.roll(x, 1, 1), pltpu.roll(x, 127, 1))
            return y + jnp.where(hi2, pltpu.roll(y, 2, 1), pltpu.roll(y, 126, 1))

        def qkv(r):
            xn = xn_v[ds(r, bm), :]
            q = _dot(xn, wt_v[pl.ds(0, D), :], NT) * qscale
            for c in range(8):
                q_s[c, :, :] = q[:, c * 128:(c + 1) * 128]
            base = pl.multiple_of(r * bm, bm) + HALO
            k = _dot(xn, wt_v[pl.ds(D, D), :], NT)
            for c in range(8):
                k_s[c, pl.ds(base, bm), :] = k[:, c * 128:(c + 1) * 128]
            v = _dot(xn, wt_v[pl.ds(2 * D, D), :], NT)
            for c in range(8):
                v_s[c, pl.ds(base, bm), :] = v[:, c * 128:(c + 1) * 128]

        groups = {1: [tuple(range(8))], 2: [(0, 1, 2, 3), (4, 5, 6, 7)], 3: [(0, 1, 2), (3, 4, 5), (6, 7)], 4: [(0, 1), (2, 3), (4, 5), (6, 7)]}[ngrp]

        def attn_qk(rb, t, g, st):
            acc = st.setdefault('acc', [None] * W)
            for c in groups[g]:
                q = q_s[c, pl.ds(t, tr), :]
                for w in range(W):
                    p = q * (rb[0][c, pl.ds(HALO + t - DIL * w, tr), :] if views else k_s[c, pl.ds(rb + (HALO + t - DIL * w), tr), :])
                    acc[w] = p if acc[w] is None else acc[w] + p

        def attn_softmax(r, t, st):
            lg = [fold(a) for a in st.pop('acc')]
            if t < DIL * (W - 1):
                row = lax.broadcasted_iota(jnp.int32, (tr, 128), 0) + (r * bm + t)
                lg = [lg[0]] + [jnp.where(row >= DIL * w, lg[w], -1e9) for w in range(1, W)]
            m = lg[0]
            for w in range(1, W):
                m = jnp.maximum(m, lg[w])
            p = [jnp.exp2(l - m) for l in lg]
            den = p[0]
            for w in range(1, W):
                den = den + p[w]
            st['p'] = p
            st['rinv'] = pltpu.reciprocal(den, approx=False, full_range=False)

        def attn_pv(rb, t, g, st):
            p = st['p']
            for c in groups[g]:
                o = None
                for w in range(W):
                    tt = p[w] * (rb[1][c, pl.ds(HALO + t - DIL * w, tr), :] if views else v_s[c, pl.ds(rb + (HALO + t - DIL * w), tr), :])
                    o = tt if o is None else o + tt
                o_s[pl.ds(t, tr), pl.ds(c * 128, 128)] = (o * st['rinv']).astype(f32 if of32 else bf16)

        def fin(r, slot):
            x = x_v[ds(r, bm), :].astype(f32)
            out_v[slot] = (x + s_s[...] * _silu(f_s[...])).astype(bf16)

        ntile = bm // tr
        def p2_body(r, _):
            rb = pl.multiple_of(r * bm, bm)
            if not fin_inline:
                fin(jnp.maximum(r - 1, 0), r)
                @pl.when(r >= 1)
                def _():
                    cp_o(r - 1, r).start()
            qkv(r)
            if views:
                rb = (k_s.at[:, pl.ds(rb, bm + HALO), :], v_s.at[:, pl.ds(rb, bm + HALO), :])
            items = []
            for t in range(ntile + lag):
                if t < ntile:
                    items += [('qk', t, g) for g in range(ngrp)]
                if t >= lag:
                    items += [('pv', t - lag, g) for g in range(ngrp)]
            nslot = ndc * slots_per
            span = nslot - slack - first
            by_slot = {}
            for i, it in enumerate(items):
                by_slot.setdefault(first + i * span // len(items), []).append(it)
            sts = [dict() for _ in range(ntile)]
            dummy = jnp.minimum(r + 8, 8)
            dummy2 = jnp.minimum(r, 7)
            acc = None
            for c in range(ndc):
                if DMARK: mark('D%d' % c)
                d = _dot(h_v[c, ds(r, bm), :], wd_v[c])
                npass = 8 * 512 // dfc if dfc >= 512 else 4
                per_pass = slots_per // npass
                for u in range(slots_per):
                    todo = by_slot.get(c * slots_per + u, [])
                    if not todo:
                        continue
                    pp, hf = u // per_pass, u % per_pass
                    col = pp * (1024 // npass)
                    anchor = d[hf * (bm // per_pass): hf * (bm // per_pass) + 8, col:col + 128]
                    kinds = set(k for k, _, _ in todo)
                    ro = 8 * ((c * slots_per + u) % 32) if rot else 0
                    if 'qk' in kinds:
                        q_s[dummy, ro:ro + 8, :] = anchor
                        if kanchor:
                            k_s[dummy2, HALO + S:HALO + S + 8, :] = anchor
                    if 'pv' in kinds:
                        if vanchor:
                            v_s[dummy2, HALO + S:HALO + S + 8, :] = anchor
                    for kind, t, g in todo:
                        if kind == 'qk':
                            attn_qk(rb, t * tr, g, sts[t])
                            if g == ngrp - 1:
                                attn_softmax(r, t * tr, sts[t])
                        else:
                            attn_pv(rb, t * tr, g, sts[t])
                acc = d if acc is None else acc + d
            if not fin_inline:
                f_s[...] = acc
            if DMARK: mark('Dend')
            if fin_inline:
                sv = _dot(o_s[...].astype(bf16), wop_v[...])
                if fin_inline == 2:
                    f_s[...] = _silu(acc)
                    out_v[r + 1] = (x_v[ds(r, bm), :].astype(f32) + sv * f_s[...]).astype(bf16)
                else:
                    out_v[r + 1] = (x_v[ds(r, bm), :].astype(f32) + sv * _silu(acc)).astype(bf16)
                cp_o(r, r + 1).start()
            else:
                s_s[...] = _dot(o_s[...].astype(bf16), wop_v[...])
            mark('M_p2end')
            return 0
        lax.fori_loop(0, nrb, p2_body, 0)
        if fin_inline:
            def wait_o():
                for r in range(nrb):
                    cp_o(r, r + 1).wait()
        else:
            fin(nrb - 1, nrb)
            cp_o(nrb - 1, nrb).start()
            def wait_o():
                for r in range(nrb):
                    cp_o(r, r + 1).wait()
        scoped('W_o', wait_o)

    return kernel


def make_fn(**cfg):
    flags = cfg.pop('flags', None)
    bm = cfg.get('bm', 256); fc = cfg.get('fc', 256); xch = cfg.get('xch', 256)
    kernel = make_kernel(**cfg)
    nrb, nfc = S // bm, F // fc
    dfc = cfg.get('dfc', 512)

    def fn(A_x, A_wqkv, A_wo, B_x, B_w_gate, B_w_up, B_w_down):
        x2 = A_x.reshape(S, D)
        anyspec = pl.BlockSpec(memory_space=pl.ANY)
        out = pl.pallas_call(
            kernel,
            out_shape=jax.ShapeDtypeStruct((S, D), bf16),
            in_specs=[anyspec] * 6,
            out_specs=anyspec,
            scratch_shapes=[
                pltpu.VMEM((S + xch, D), bf16),
                pltpu.VMEM((S + xch, D), bf16),
                pltpu.VMEM((NP + 1, D, 128), bf16),
                pltpu.VMEM((D + 64, D), bf16),
                pltpu.VMEM((nfc, D, fc), bf16),
                pltpu.VMEM((nfc, D, fc), bf16),
                pltpu.VMEM((F // dfc, dfc, D), bf16),
                pltpu.VMEM((3 * D, D), bf16),
                pltpu.VMEM((D, D), bf16),
                pltpu.VMEM((F // dfc, S, dfc), bf16),
                pltpu.VMEM((9, bm, 128), f32),
                pltpu.VMEM((8, HALO + S + KPAD, 128), f32),
                pltpu.VMEM((8, HALO + S + KPAD, 128), f32),
                pltpu.VMEM((bm, D), f32 if cfg.get('of32', False) else bf16),
                pltpu.VMEM((bm, D), f32),
                pltpu.VMEM((bm, D), f32),
                pltpu.VMEM((nrb + 1, bm, D), bf16),
                pltpu.SemaphoreType.DMA((S // xch,)),
                pltpu.SemaphoreType.DMA((nfc,)),
                pltpu.SemaphoreType.DMA((nfc,)),
                pltpu.SemaphoreType.DMA((nfc,)),
                pltpu.SemaphoreType.DMA((NP + 1,)),
                pltpu.SemaphoreType.DMA((nrb,)),
                pltpu.SemaphoreType.DMA((4,)),
            ],
            compiler_params=pltpu.CompilerParams(vmem_limit_bytes=120 * 1024 * 1024, disable_bounds_checks=True, disable_semaphore_checks=True, **({'flags': flags} if flags else {})),
        )(x2, A_wqkv, A_wo, B_w_gate, B_w_up, B_w_down)
        return out.reshape(1, S, D)
    return fn


_FN = make_fn(bm=256, bg=1024, fc=256, ngrp=2, slack=27, g0split=(144, 0, 112))


@jax.jit
def pallas_recurrent_scan__sliding_local_dilated__swiglu_ffn__prompt_kernel(
    A_x, A_wqkv, A_wo, B_x, B_w_gate, B_w_up, B_w_down,
):
    return _FN(A_x, A_wqkv, A_wo, B_x, B_w_gate, B_w_up, B_w_down)
```

```python
import jax
import jax.numpy as jnp
from jax import lax
from jax.experimental import pallas as pl
from jax.experimental.pallas import tpu as pltpu

S, D, F = 2048, 1024, 3584
H, DH, W, DIL = 32, 32, 8, 2
HALO = 16
KPAD = 16
NP = 3 * D // 128
BM = 256
NRB = S // BM
FC = 256
NFC = F // FC
DFC = 512
NDC = F // DFC
BG = 1024
TR = 16
LN_STEP = 16
LN_SPLIT = 144
LOG2E = 1.4426950408889634
SLOTS_PER, SLOT_FIRST, SLOT_SLACK = 16, 2, 34
QK_GROUPS = ((0, 1, 2, 3, 4), (5, 6, 7))
PV_GROUPS = ((0, 1, 2, 3), (4, 5, 6, 7))

f32, bf16 = jnp.float32, jnp.bfloat16
NN = (((1,), (0,)), ((), ()))
NT = (((1,), (1,)), ((), ()))


def _dot(a, b, dn=NN):
    return lax.dot_general(a, b, dn, preferred_element_type=f32)


def _silu(x):
    e = jnp.exp2(jnp.minimum(x * (-LOG2E), 126.0))
    return x * pltpu.reciprocal(1.0 + e, approx=False, full_range=False)


def _ds(i, n):
    return pl.ds(i * n, n) if isinstance(i, int) else pl.ds(pl.multiple_of(i * n, n), n)


def _kernel(x_hbm, wqkv_hbm, wo_hbm, wg_hbm, wu_hbm, wd_hbm, o_hbm,
            x_v, xn_v, wqkv_v, wo_v, wg_v, wu_v, wd_v, wt_v, wop_v,
            h_v, q_s, k_s, v_s, o_s, out_v,
            sem_x, sem_g, sem_u, sem_d, sem_a, sem_o):
    def cp_x(r):
        return pltpu.make_async_copy(x_hbm.at[_ds(r, BM), :], x_v.at[_ds(r, BM), :], sem_x.at[r])

    def cp_g(c):
        return pltpu.make_async_copy(wg_hbm.at[:, _ds(c, FC)], wg_v.at[c], sem_g.at[c])

    def cp_u(c):
        return pltpu.make_async_copy(wu_hbm.at[:, _ds(c, FC)], wu_v.at[c], sem_u.at[c])

    def cp_d(n):
        return pltpu.make_async_copy(wd_hbm.at[:, _ds(n, 128)], wd_v.at[n], sem_d.at[n])

    def cp_a(p):
        return pltpu.make_async_copy(wqkv_hbm.at[:, _ds(p, 128)], wqkv_v.at[p], sem_a.at[p])

    def cp_wo():
        return pltpu.make_async_copy(wo_hbm, wo_v.at[pl.ds(0, D), :], sem_a.at[NP])

    def cp_o(r):
        return pltpu.make_async_copy(out_v.at[r], o_hbm.at[_ds(r, BM), :], sem_o.at[r])

    def layernorm(base, off, n):
        for t in range(off, off + n, LN_STEP):
            rows = pl.ds(base + t if isinstance(base, int) else pl.multiple_of(base + t, LN_STEP), LN_STEP)
            x = x_v[rows, :].astype(f32)
            m = jnp.mean(x, axis=-1, keepdims=True)
            xc = x - m
            var = jnp.mean(xc * xc, axis=-1, keepdims=True)
            xn_v[rows, :] = (xc * lax.rsqrt(var + 1e-5)).astype(bf16)

    def swiglu(g, u):
        return (_silu(g) * u).astype(bf16)

    sub_i = lax.broadcasted_iota(jnp.int32, (8, 128), 0)
    lo4 = sub_i < 4
    lo2 = (sub_i % 4) < 2

    def regroup_rows(t):
        tu = pltpu.bitcast(t, jnp.uint32)

        def stage(a, b, sh, m):
            return jnp.where(m, a, pltpu.roll(b, sh, 0)), jnp.where(m, pltpu.roll(a, 8 - sh, 0), b)

        outs = []
        for b in range(2):
            v = [tu[hl * 16 + 8 * b: hl * 16 + 8 * b + 8, :] for hl in range(4)]
            a0, a2 = stage(v[0], v[2], 4, lo4)
            a1, a3 = stage(v[1], v[3], 4, lo4)
            b0, b1 = stage(a0, a1, 2, lo2)
            b2, b3 = stage(a2, a3, 2, lo2)
            outs += [pltpu.bitcast(z, bf16) for z in (b0, b1, b2, b3)]
        return outs

    def permute_strip(p, kt):
        blocks = regroup_rows(wqkv_v[p, pl.ds(kt * 128, 128), :].T)
        m, i = p // 8, p % 8
        for c in range(8):
            o = pl.multiple_of(m * D + c * 128 + 16 * i, 16)
            wt_v[pl.ds(o, 16), pl.ds(kt * 128, 128)] = blocks[c]

    def permute_wo(i, nt):
        blocks = regroup_rows(wo_v[_ds(i, 128), pl.ds(nt * 128, 128)])
        for c in range(8):
            o = pl.multiple_of(c * 128 + 16 * i, 16)
            wop_v[pl.ds(o, 16), pl.ds(nt * 128, 128)] = blocks[c]

    cp_x(0).start(); cp_g(0).start(); cp_u(0).start()
    for c in range(8):
        k_s[c, pl.ds(0, HALO), :] = jnp.zeros((HALO, 128), f32)
        v_s[c, pl.ds(0, HALO), :] = jnp.zeros((HALO, 128), f32)
    x_v[pl.ds(S, BM), :] = jnp.zeros((BM, D), bf16)
    cp_x(0).wait()
    cp_x(1).start()
    layernorm(0, 0, BM)
    cp_g(0).wait()
    g = _dot(xn_v[pl.ds(0, BM), :], wg_v[0])
    cp_u(0).wait()
    cp_x(2).start()
    u = _dot(xn_v[pl.ds(0, BM), :], wu_v[0])
    h_v[0, pl.ds(0, BM), pl.ds(0, FC)] = swiglu(g, u)
    cp_x(1).wait()
    layernorm(BM, 0, BM)
    cp_x(3).start()

    def g0_body(r, _):
        @pl.when(r + 3 < NRB)
        def _():
            cp_x(r + 3).start()

        @pl.when(r == 5)
        def _():
            cp_wo().start()

        @pl.when(r == 4)
        def _():
            cp_g(1).start(); cp_u(1).start()
            cp_a(0).start(); cp_a(1).start()

        @pl.when(r + 1 < NRB)
        def _():
            cp_x(r + 1).wait()

        base = pl.multiple_of(r * BM, BM)
        rows = pl.ds(base, BM)
        g = _dot(xn_v[rows, :], wg_v[0, :, pl.ds(0, 128)])
        u = _dot(xn_v[rows, :], wu_v[0, :, pl.ds(0, 128)])
        h_v[0, rows, pl.ds(0, 128)] = swiglu(g, u)
        layernorm(base, BM, LN_SPLIT)
        g = _dot(xn_v[rows, :], wg_v[0, :, pl.ds(128, 128)])
        u = _dot(xn_v[rows, :], wu_v[0, :, pl.ds(128, 128)])
        h_v[0, rows, pl.ds(128, 128)] = swiglu(g, u)
        layernorm(base, BM + LN_SPLIT, BM - LN_SPLIT)
        return 0

    lax.fori_loop(1, NRB, g0_body, 0)

    jobs = []
    for kt in range(8):
        jobs += [('a', 0, kt), ('a', 1, kt), ('o', 0, kt)]
    nblk = S // BG
    cuts = [len(jobs) * i // (nblk - 1) for i in range(nblk)] + [len(jobs)]

    def g_body(c, _):
        j = c - 1
        p0 = jnp.maximum(2 * j - 2, 0)
        cp_g(c).wait(); cp_u(c).wait()

        @pl.when(j == 0)
        def _():
            cp_wo().wait()

        @pl.when(j != 1)
        def _():
            cp_a(p0).wait(); cp_a(p0 + 1).wait()

        @pl.when(c + 1 < NFC)
        def _():
            cp_g(c + 1).start(); cp_u(c + 1).start()

        @pl.when(jnp.logical_and(j >= 1, 2 * j < NP))
        def _():
            cp_a(2 * j).start(); cp_a(2 * j + 1).start()

        @pl.when(j < 8)
        def _():
            cp_d(j).start()

        da = jnp.minimum(c + NP, NP)
        do = pl.multiple_of(jnp.minimum(c + 64, 64) * 16, 16)
        for ib in range(nblk):
            rows = pl.ds(ib * BG, BG)
            xn = xn_v[rows, :]
            hh = swiglu(_dot(xn, wg_v[c]), _dot(xn, wu_v[c]))
            h_v[c // 2, rows, _ds(c % 2, FC)] = hh
            mine = jobs[cuts[ib]:cuts[ib + 1]]
            for n, (kind, dp, kt) in enumerate(mine):
                ar = (n * BG // len(mine)) // 16 * 16
                anchor = hh[ar:ar + 16, 0:128]
                if kind == 'a':
                    wqkv_v[da, 0:16, :] = anchor
                    permute_strip(p0 + dp, kt)
                else:
                    wo_v[pl.ds(do, 16), 0:128] = anchor
                    permute_wo(jnp.minimum(j, 7), kt)
        return 0

    assert 2 * (NFC - 2) >= NP and NFC - 1 >= 8 and DFC == 2 * FC
    lax.fori_loop(1, NFC, g_body, 0)
    for n in range(8):
        cp_d(n).wait()

    qscale = (DH ** -0.5) * LOG2E
    lane = lax.broadcasted_iota(jnp.int32, (TR, 128), 1)
    odd = (lane % 2) == 1
    hi2 = (lane % 4) >= 2

    def fold(x):
        y = x + jnp.where(odd, pltpu.roll(x, 1, 1), pltpu.roll(x, 127, 1))
        return y + jnp.where(hi2, pltpu.roll(y, 2, 1), pltpu.roll(y, 126, 1))

    def project(r):
        xn = xn_v[_ds(r, BM), :]
        base = pl.multiple_of(r * BM, BM) + HALO
        v = _dot(xn, wt_v[pl.ds(2 * D, D), :], NT)
        for c in range(8):
            v_s[c, pl.ds(base, BM), :] = v[:, c * 128:(c + 1) * 128]
        k = _dot(xn, wt_v[pl.ds(D, D), :], NT)
        for c in range(8):
            k_s[c, pl.ds(base, BM), :] = k[:, c * 128:(c + 1) * 128]
        q = _dot(xn, wt_v[pl.ds(0, D), :], NT) * qscale
        for c in range(8):
            q_s[c, :, :] = q[:, c * 128:(c + 1) * 128]

    def attn_qk(rb, t, chunks, st):
        acc = st.setdefault('acc', [None] * W)
        for c in chunks:
            q = q_s[c, pl.ds(t, TR), :]
            for w in range(W):
                p = q * k_s[c, pl.ds(rb + (HALO + t - DIL * w), TR), :]
                acc[w] = p if acc[w] is None else acc[w] + p

    def attn_softmax(rb, t, st):
        lg = [fold(a) for a in st.pop('acc')]
        if t < DIL * (W - 1):
            row = lax.broadcasted_iota(jnp.int32, (TR, 128), 0) + (rb + t)
            lg = [lg[0]] + [jnp.where(row >= DIL * w, lg[w], -1e9) for w in range(1, W)]
        m = lg[0]
        for w in range(1, W):
            m = jnp.maximum(m, lg[w])
        p = [jnp.exp2(l - m) for l in lg]
        den = p[0]
        for w in range(1, W):
            den = den + p[w]
        st['p'] = p
        st['rinv'] = pltpu.reciprocal(den, approx=False, full_range=False)

    def attn_pv(rb, t, chunks, st):
        p = st['p']
        for c in chunks:
            o = None
            for w in range(W):
                tt = p[w] * v_s[c, pl.ds(rb + (HALO + t - DIL * w), TR), :]
                o = tt if o is None else o + tt
            o_s[pl.ds(t, TR), pl.ds(c * 128, 128)] = (o * st['rinv']).astype(bf16)

    ntile = BM // TR
    items = []
    for t in range(ntile + 1):
        if t < ntile:
            items += [('qk', t, g) for g in range(len(QK_GROUPS))]
        if t >= 1:
            items += [('pv', t - 1, g) for g in range(len(PV_GROUPS))]
    span = NDC * SLOTS_PER - SLOT_SLACK - SLOT_FIRST
    by_slot = {}
    for i, it in enumerate(items):
        by_slot.setdefault(SLOT_FIRST + i * span // len(items), []).append(it)

    def r_body(r, _):
        rb = pl.multiple_of(r * BM, BM)
        project(r)
        dq = jnp.minimum(r + 8, 8)
        dkv = jnp.minimum(r, 7)
        sts = [dict() for _ in range(ntile)]
        acc = None
        for c in range(NDC):
            wd = jnp.concatenate([wd_v[n, pl.ds(c * DFC, DFC), :] for n in range(8)], axis=1)
            d = _dot(h_v[c, _ds(r, BM), :], wd)
            for u in range(SLOTS_PER):
                todo = by_slot.get(c * SLOTS_PER + u, [])
                if not todo:
                    continue
                col, row = (u // 2) * 128, (u % 2) * (BM // 2)
                anchor = d[row:row + 8, col:col + 128]
                ro = 8 * ((c * SLOTS_PER + u) % 32)
                kinds = set(k for k, _, _ in todo)
                if 'qk' in kinds:
                    q_s[dq, ro:ro + 8, :] = anchor
                    k_s[dkv, HALO + S:HALO + S + 8, :] = anchor
                if 'pv' in kinds:
                    v_s[dkv, HALO + S:HALO + S + 8, :] = anchor
                for kind, t, g in todo:
                    if kind == 'qk':
                        attn_qk(rb, t * TR, QK_GROUPS[g], sts[t])
                        if g == len(QK_GROUPS) - 1:
                            attn_softmax(rb, t * TR, sts[t])
                    else:
                        attn_pv(rb, t * TR, PV_GROUPS[g], sts[t])
            acc = d if acc is None else acc + d
        s = _dot(o_s[...], wop_v[...])
        out_v[r] = (x_v[_ds(r, BM), :].astype(f32) + s * _silu(acc)).astype(bf16)
        cp_o(r).start()
        return 0

    lax.fori_loop(0, NRB, r_body, 0)
    for r in range(NRB):
        cp_o(r).wait()


@jax.jit
def pallas_recurrent_scan__sliding_local_dilated__swiglu_ffn__prompt_kernel(
    A_x, A_wqkv, A_wo, B_x, B_w_gate, B_w_up, B_w_down,
):
    del B_x
    anyspec = pl.BlockSpec(memory_space=pl.ANY)
    out = pl.pallas_call(
        _kernel,
        out_shape=jax.ShapeDtypeStruct((S, D), bf16),
        in_specs=[anyspec] * 6,
        out_specs=anyspec,
        scratch_shapes=[
            pltpu.VMEM((S + BM, D), bf16),
            pltpu.VMEM((S + BM, D), bf16),
            pltpu.VMEM((NP + 1, D, 128), bf16),
            pltpu.VMEM((D + 64, D), bf16),
            pltpu.VMEM((NFC, D, FC), bf16),
            pltpu.VMEM((NFC, D, FC), bf16),
            pltpu.VMEM((8, F, 128), bf16),
            pltpu.VMEM((3 * D, D), bf16),
            pltpu.VMEM((D, D), bf16),
            pltpu.VMEM((NDC, S, DFC), bf16),
            pltpu.VMEM((9, BM, 128), f32),
            pltpu.VMEM((8, HALO + S + KPAD, 128), f32),
            pltpu.VMEM((8, HALO + S + KPAD, 128), f32),
            pltpu.VMEM((BM, D), bf16),
            pltpu.VMEM((NRB, BM, D), bf16),
            pltpu.SemaphoreType.DMA((NRB,)),
            pltpu.SemaphoreType.DMA((NFC,)),
            pltpu.SemaphoreType.DMA((NFC,)),
            pltpu.SemaphoreType.DMA((8,)),
            pltpu.SemaphoreType.DMA((NP + 1,)),
            pltpu.SemaphoreType.DMA((NRB,)),
        ],
        compiler_params=pltpu.CompilerParams(
            vmem_limit_bytes=120 * 1024 * 1024,
            disable_bounds_checks=True,
            disable_semaphore_checks=True,
        ),
    )(A_x.reshape(S, D), A_wqkv, A_wo, B_w_gate, B_w_up, B_w_down)
    return out.reshape(1, S, D)
```

```python
import jax
import jax.numpy as jnp
from jax import lax
from jax.experimental import pallas as pl
from jax.experimental.pallas import tpu as pltpu

S, D, F = 2048, 1024, 3584
H, DH, W, DIL = 32, 32, 8, 2
HALO = 16
KPAD = 16
NP = 3 * D // 128
BM = 256
NRB = S // BM
FC = 256
NFC = F // FC
DFC = 512
NDC = F // DFC
BG = 1024
TR = 16
LN_STEP = 16
LN_SPLIT = 64
LOG2E = 1.4426950408889634
SLOTS_PER, SLOT_FIRST, SLOT_SLACK = 16, 0, 26
QK_GROUPS = ((0, 1, 2, 3, 4), (5, 6, 7))
PV_GROUPS = ((0, 1, 2, 3), (4, 5, 6, 7))

f32, bf16 = jnp.float32, jnp.bfloat16
NN = (((1,), (0,)), ((), ()))
NT = (((1,), (1,)), ((), ()))


def _dot(a, b, dn=NN):
    return lax.dot_general(a, b, dn, preferred_element_type=f32)


def _silu(x):
    e = jnp.exp2(jnp.minimum(x * (-LOG2E), 126.0))
    return x * pltpu.reciprocal(1.0 + e, approx=False, full_range=False)


def _ds(i, n):
    return pl.ds(i * n, n) if isinstance(i, int) else pl.ds(pl.multiple_of(i * n, n), n)


def _kernel(x_hbm, wqkv_hbm, wo_hbm, wg_hbm, wu_hbm, wd_hbm, o_hbm,
            x_v, xn_v, wqkv_v, wo_v, wg_v, wu_v, wd_v, wt_v, wop_v,
            h_v, q_s, k_s, v_s, o_s, out_v,
            sem_x, sem_g, sem_u, sem_d, sem_a, sem_o):
    def cp_x(r):
        return pltpu.make_async_copy(x_hbm.at[_ds(r, BM), :], x_v.at[_ds(r, BM), :], sem_x.at[r])

    def cp_g(c):
        return pltpu.make_async_copy(wg_hbm.at[:, _ds(c, FC)], wg_v.at[c], sem_g.at[c])

    def cp_u(c):
        return pltpu.make_async_copy(wu_hbm.at[:, _ds(c, FC)], wu_v.at[c], sem_u.at[c])

    def cp_d(n):
        return pltpu.make_async_copy(wd_hbm.at[:, _ds(n, 128)], wd_v.at[n], sem_d.at[n])

    def cp_a(p):
        return pltpu.make_async_copy(wqkv_hbm.at[:, _ds(p, 128)], wqkv_v.at[p], sem_a.at[p])

    def cp_wo():
        return pltpu.make_async_copy(wo_hbm, wo_v.at[pl.ds(0, D), :], sem_a.at[NP])

    def cp_o(r):
        return pltpu.make_async_copy(out_v.at[r], o_hbm.at[_ds(r, BM), :], sem_o.at[r])

    def layernorm(base, off, n):
        for t in range(off, off + n, LN_STEP):
            rows = pl.ds(base + t if isinstance(base, int) else pl.multiple_of(base + t, LN_STEP), LN_STEP)
            x = x_v[rows, :].astype(f32)
            m = jnp.mean(x, axis=-1, keepdims=True)
            xc = x - m
            var = jnp.mean(xc * xc, axis=-1, keepdims=True)
            xn_v[rows, :] = (xc * lax.rsqrt(var + 1e-5)).astype(bf16)

    def swiglu(g, u):
        return (_silu(g) * u).astype(bf16)

    sub_i = lax.broadcasted_iota(jnp.int32, (8, 128), 0)
    lo4 = sub_i < 4
    lo2 = (sub_i % 4) < 2

    def regroup_rows(t):
        tu = pltpu.bitcast(t, jnp.uint32)

        def stage(a, b, sh, m):
            return jnp.where(m, a, pltpu.roll(b, sh, 0)), jnp.where(m, pltpu.roll(a, 8 - sh, 0), b)

        outs = []
        for b in range(2):
            v = [tu[hl * 16 + 8 * b: hl * 16 + 8 * b + 8, :] for hl in range(4)]
            a0, a2 = stage(v[0], v[2], 4, lo4)
            a1, a3 = stage(v[1], v[3], 4, lo4)
            b0, b1 = stage(a0, a1, 2, lo2)
            b2, b3 = stage(a2, a3, 2, lo2)
            outs += [pltpu.bitcast(z, bf16) for z in (b0, b1, b2, b3)]
        return outs

    def permute_strip(p, kt):
        blocks = regroup_rows(wqkv_v[p, pl.ds(kt * 128, 128), :].T)
        m, i = p // 8, p % 8
        for c in range(8):
            o = pl.multiple_of(m * D + c * 128 + 16 * i, 16)
            wt_v[pl.ds(o, 16), pl.ds(kt * 128, 128)] = blocks[c]

    def permute_wo(i, nt):
        blocks = regroup_rows(wo_v[_ds(i, 128), pl.ds(nt * 128, 128)])
        for c in range(8):
            o = pl.multiple_of(c * 128 + 16 * i, 16)
            wop_v[pl.ds(o, 16), pl.ds(nt * 128, 128)] = blocks[c]

    cp_x(0).start(); cp_g(0).start(); cp_u(0).start()
    for c in range(8):
        k_s[c, pl.ds(0, HALO), :] = jnp.zeros((HALO, 128), f32)
        v_s[c, pl.ds(0, HALO), :] = jnp.zeros((HALO, 128), f32)
    x_v[pl.ds(S, BM), :] = jnp.zeros((BM, D), bf16)
    cp_x(0).wait()
    cp_x(1).start()
    layernorm(0, 0, BM)
    cp_g(0).wait()
    g = _dot(xn_v[pl.ds(0, BM), :], wg_v[0])
    cp_u(0).wait()
    cp_x(2).start()
    u = _dot(xn_v[pl.ds(0, BM), :], wu_v[0])
    h_v[0, pl.ds(0, BM), pl.ds(0, FC)] = swiglu(g, u)
    cp_x(1).wait()
    layernorm(BM, 0, BM)
    cp_x(3).start(); cp_x(4).start()

    def g0_body(r, _):
        @pl.when(r + 4 < NRB)
        def _():
            cp_x(r + 4).start()

        @pl.when(r == 5)
        def _():
            cp_wo().start()

        @pl.when(r == 4)
        def _():
            cp_g(1).start(); cp_u(1).start()
            cp_a(0).start(); cp_a(1).start()

        @pl.when(r + 1 < NRB)
        def _():
            cp_x(r + 1).wait()

        base = pl.multiple_of(r * BM, BM)
        rows = pl.ds(base, BM)
        g = _dot(xn_v[rows, :], wg_v[0, :, pl.ds(0, 128)])
        u = _dot(xn_v[rows, :], wu_v[0, :, pl.ds(0, 128)])
        h_v[0, rows, pl.ds(0, 128)] = swiglu(g, u)
        layernorm(base, BM, LN_SPLIT)
        g = _dot(xn_v[rows, :], wg_v[0, :, pl.ds(128, 128)])
        u = _dot(xn_v[rows, :], wu_v[0, :, pl.ds(128, 128)])
        h_v[0, rows, pl.ds(128, 128)] = swiglu(g, u)
        layernorm(base, BM + LN_SPLIT, BM - LN_SPLIT)
        return 0

    lax.fori_loop(1, NRB, g0_body, 0)

    jobs = []
    for kt in range(8):
        jobs += [('a', 0, kt), ('a', 1, kt), ('o', 0, kt)]
    nblk = S // BG
    cuts = [len(jobs) * i // (nblk - 1) for i in range(nblk)] + [len(jobs)]

    def g_body(c, _):
        j = c - 1
        p0 = jnp.maximum(2 * j - 2, 0)
        cp_g(c).wait(); cp_u(c).wait()

        @pl.when(j == 0)
        def _():
            cp_wo().wait()

        @pl.when(j != 1)
        def _():
            cp_a(p0).wait(); cp_a(p0 + 1).wait()

        @pl.when(c + 1 < NFC)
        def _():
            cp_g(c + 1).start(); cp_u(c + 1).start()

        @pl.when(jnp.logical_and(j >= 1, 2 * j < NP))
        def _():
            cp_a(2 * j).start(); cp_a(2 * j + 1).start()

        @pl.when(j < 8)
        def _():
            cp_d(j).start()

        da = jnp.minimum(c + NP, NP)
        do = pl.multiple_of(jnp.minimum(c + 64, 64) * 16, 16)
        for ib in range(nblk):
            rows = pl.ds(ib * BG, BG)
            xn = xn_v[rows, :]
            hh = swiglu(_dot(xn, wg_v[c]), _dot(xn, wu_v[c]))
            h_v[c // 2, rows, _ds(c % 2, FC)] = hh
            mine = jobs[cuts[ib]:cuts[ib + 1]]
            for n, (kind, dp, kt) in enumerate(mine):
                ar = (n * BG // len(mine)) // 16 * 16
                anchor = hh[ar:ar + 16, 0:128]
                if kind == 'a':
                    wqkv_v[da, 0:16, :] = anchor
                    permute_strip(p0 + dp, kt)
                else:
                    wo_v[pl.ds(do, 16), 0:128] = anchor
                    permute_wo(jnp.minimum(j, 7), kt)
        return 0

    assert 2 * (NFC - 2) >= NP and NFC - 1 >= 8 and DFC == 2 * FC
    lax.fori_loop(1, NFC, g_body, 0)
    for n in range(8):
        cp_d(n).wait()

    qscale = (DH ** -0.5) * LOG2E
    lane = lax.broadcasted_iota(jnp.int32, (TR, 128), 1)
    odd = (lane % 2) == 1
    hi2 = (lane % 4) >= 2

    def fold(x):
        y = x + jnp.where(odd, pltpu.roll(x, 1, 1), pltpu.roll(x, 127, 1))
        return y + jnp.where(hi2, pltpu.roll(y, 2, 1), pltpu.roll(y, 126, 1))

    def project(r):
        xn = xn_v[_ds(r, BM), :]
        base = pl.multiple_of(r * BM, BM) + HALO
        v = _dot(xn, wt_v[pl.ds(2 * D, D), :], NT)
        for c in range(8):
            v_s[c, pl.ds(base, BM), :] = v[:, c * 128:(c + 1) * 128]
        k = _dot(xn, wt_v[pl.ds(D, D), :], NT)
        for c in range(8):
            k_s[c, pl.ds(base, BM), :] = k[:, c * 128:(c + 1) * 128]
        q = _dot(xn, wt_v[pl.ds(0, D), :], NT) * qscale
        for c in range(8):
            q_s[c, :, :] = q[:, c * 128:(c + 1) * 128]

    def attn_qk(rb, t, chunks, st):
        acc = st.setdefault('acc', [None] * W)
        for c in chunks:
            q = q_s[c, pl.ds(t, TR), :]
            for w in range(W):
                p = q * k_s[c, pl.ds(rb + (HALO + t - DIL * w), TR), :]
                acc[w] = p if acc[w] is None else acc[w] + p

    def attn_softmax(rb, t, st):
        lg = [fold(a) for a in st.pop('acc')]
        if t < DIL * (W - 1):
            row = lax.broadcasted_iota(jnp.int32, (TR, 128), 0) + (rb + t)
            lg = [lg[0]] + [jnp.where(row >= DIL * w, lg[w], -1e9) for w in range(1, W)]
        m = lg[0]
        for w in range(1, W):
            m = jnp.maximum(m, lg[w])
        p = [jnp.exp2(l - m) for l in lg]
        den = p[0]
        for w in range(1, W):
            den = den + p[w]
        st['p'] = p
        st['rinv'] = pltpu.reciprocal(den, approx=False, full_range=False)

    def attn_pv(rb, t, chunks, st):
        p = st['p']
        for c in chunks:
            o = None
            for w in range(W):
                tt = p[w] * v_s[c, pl.ds(rb + (HALO + t - DIL * w), TR), :]
                o = tt if o is None else o + tt
            o_s[pl.ds(t, TR), pl.ds(c * 128, 128)] = (o * st['rinv']).astype(bf16)

    ntile = BM // TR
    items = []
    for t in range(ntile + 1):
        if t < ntile:
            items += [('qk', t, g) for g in range(len(QK_GROUPS))]
        if t >= 1:
            items += [('pv', t - 1, g) for g in range(len(PV_GROUPS))]
    span = NDC * SLOTS_PER - SLOT_SLACK - SLOT_FIRST
    by_slot = {}
    for i, it in enumerate(items):
        by_slot.setdefault(SLOT_FIRST + i * span // len(items), []).append(it)

    def r_body(r, _):
        rb = pl.multiple_of(r * BM, BM)
        project(r)
        dq = jnp.minimum(r + 8, 8)
        dkv = jnp.minimum(r, 7)
        sts = [dict() for _ in range(ntile)]
        acc = None
        for c in range(NDC):
            wd = jnp.concatenate([wd_v[n, pl.ds(c * DFC, DFC), :] for n in range(8)], axis=1)
            d = _dot(h_v[c, _ds(r, BM), :], wd)
            for u in range(SLOTS_PER):
                todo = by_slot.get(c * SLOTS_PER + u, [])
                if not todo:
                    continue
                col, row = (u // 2) * 128, (u % 2) * (BM // 2)
                anchor = d[row:row + 8, col:col + 128]
                ro = 8 * ((c * SLOTS_PER + u) % 32)
                kinds = set(k for k, _, _ in todo)
                if 'qk' in kinds:
                    q_s[dq, ro:ro + 8, :] = anchor
                    k_s[dkv, HALO + S:HALO + S + 8, :] = anchor
                if 'pv' in kinds:
                    v_s[dkv, HALO + S:HALO + S + 8, :] = anchor
                for kind, t, g in todo:
                    if kind == 'qk':
                        attn_qk(rb, t * TR, QK_GROUPS[g], sts[t])
                        if g == len(QK_GROUPS) - 1:
                            attn_softmax(rb, t * TR, sts[t])
                    else:
                        attn_pv(rb, t * TR, PV_GROUPS[g], sts[t])
            acc = d if acc is None else acc + d
        s = _dot(o_s[...], wop_v[...])
        out_v[r] = (x_v[_ds(r, BM), :].astype(f32) + s * _silu(acc)).astype(bf16)
        cp_o(r).start()
        return 0

    lax.fori_loop(0, NRB, r_body, 0)
    for r in range(NRB):
        cp_o(r).wait()


@jax.jit
def pallas_recurrent_scan__sliding_local_dilated__swiglu_ffn__prompt_kernel(
    A_x, A_wqkv, A_wo, B_x, B_w_gate, B_w_up, B_w_down,
):
    del B_x
    anyspec = pl.BlockSpec(memory_space=pl.ANY)
    out = pl.pallas_call(
        _kernel,
        out_shape=jax.ShapeDtypeStruct((S, D), bf16),
        in_specs=[anyspec] * 6,
        out_specs=anyspec,
        scratch_shapes=[
            pltpu.VMEM((S + BM, D), bf16),
            pltpu.VMEM((S + BM, D), bf16),
            pltpu.VMEM((NP + 1, D, 128), bf16),
            pltpu.VMEM((D + 64, D), bf16),
            pltpu.VMEM((NFC, D, FC), bf16),
            pltpu.VMEM((NFC, D, FC), bf16),
            pltpu.VMEM((8, F, 128), bf16),
            pltpu.VMEM((3 * D, D), bf16),
            pltpu.VMEM((D, D), bf16),
            pltpu.VMEM((NDC, S, DFC), bf16),
            pltpu.VMEM((9, BM, 128), f32),
            pltpu.VMEM((8, HALO + S + KPAD, 128), f32),
            pltpu.VMEM((8, HALO + S + KPAD, 128), f32),
            pltpu.VMEM((BM, D), bf16),
            pltpu.VMEM((NRB, BM, D), bf16),
            pltpu.SemaphoreType.DMA((NRB,)),
            pltpu.SemaphoreType.DMA((NFC,)),
            pltpu.SemaphoreType.DMA((NFC,)),
            pltpu.SemaphoreType.DMA((8,)),
            pltpu.SemaphoreType.DMA((NP + 1,)),
            pltpu.SemaphoreType.DMA((NRB,)),
        ],
        compiler_params=pltpu.CompilerParams(
            vmem_limit_bytes=120 * 1024 * 1024,
            disable_bounds_checks=True,
            disable_semaphore_checks=True,
            flags={'XLA_TPU_EVENLY_DISTRIBUTE_CRITICAL_NODES': True},
        ),
    )(A_x.reshape(S, D), A_wqkv, A_wo, B_w_gate, B_w_up, B_w_down)
    return out.reshape(1, S, D)
```

```python
import jax
import jax.numpy as jnp
from jax import lax
from jax.experimental import pallas as pl
from jax.experimental.pallas import tpu as pltpu

S, D, F = 2048, 1024, 3584
H, DH, W, DIL = 32, 32, 8, 2
HALO = 16
KPAD = 16
NP = 3 * D // 128
BM = 256
NRB = S // BM
FC = 256
NFC = F // FC
DFC = 512
NDC = F // DFC
BG = 1024
TR = 16
LN_STEP = 16
LN_SPLIT = 64
LOG2E = 1.4426950408889634
SLOTS_PER, SLOT_FIRST, SLOT_SLACK = 16, 0, 26
QK_GROUPS = ((0, 1, 2, 3, 4), (5, 6, 7))
PV_GROUPS = ((0, 1, 2, 3), (4, 5, 6, 7))

f32, bf16 = jnp.float32, jnp.bfloat16
NN = (((1,), (0,)), ((), ()))
NT = (((1,), (1,)), ((), ()))


def _dot(a, b, dn=NN):
    return lax.dot_general(a, b, dn, preferred_element_type=f32)


def _silu(x):
    e = jnp.exp2(jnp.minimum(x * (-LOG2E), 126.0))
    return x * pltpu.reciprocal(1.0 + e, approx=False, full_range=False)


def _ds(i, n):
    return pl.ds(i * n, n) if isinstance(i, int) else pl.ds(pl.multiple_of(i * n, n), n)


def _kernel(x_hbm, wqkv_hbm, wo_hbm, wg_hbm, wu_hbm, wd_hbm, o_hbm,
            x_v, xn_v, wqkv_v, wo_v, wg_v, wu_v, wd_v, wt_v, wop_v,
            h_v, q_s, k_s, v_s, o_s, out_v,
            sem_x, sem_g, sem_u, sem_d, sem_a, sem_o):
    def cp_x(r):
        return pltpu.make_async_copy(x_hbm.at[_ds(r, BM), :], x_v.at[_ds(r, BM), :], sem_x.at[r])

    def cp_g(c):
        return pltpu.make_async_copy(wg_hbm.at[:, _ds(c, FC)], wg_v.at[c], sem_g.at[c])

    def cp_u(c):
        return pltpu.make_async_copy(wu_hbm.at[:, _ds(c, FC)], wu_v.at[c], sem_u.at[c])

    def cp_d(n):
        return pltpu.make_async_copy(wd_hbm.at[:, _ds(n, 128)], wd_v.at[n], sem_d.at[n])

    def cp_a(p):
        return pltpu.make_async_copy(wqkv_hbm.at[:, _ds(p, 128)], wqkv_v.at[p], sem_a.at[p])

    def cp_wo():
        return pltpu.make_async_copy(wo_hbm, wo_v.at[pl.ds(0, D), :], sem_a.at[NP])

    def cp_o(r):
        return pltpu.make_async_copy(out_v.at[r], o_hbm.at[_ds(r, BM), :], sem_o.at[r])

    def layernorm(base, off, n):
        for t in range(off, off + n, LN_STEP):
            rows = pl.ds(base + t if isinstance(base, int) else pl.multiple_of(base + t, LN_STEP), LN_STEP)
            x = x_v[rows, :].astype(f32)
            m = jnp.mean(x, axis=-1, keepdims=True)
            xc = x - m
            var = jnp.mean(xc * xc, axis=-1, keepdims=True)
            xn_v[rows, :] = (xc * lax.rsqrt(var + 1e-5)).astype(bf16)

    def swiglu(g, u):
        return (_silu(g) * u).astype(bf16)

    sub_i = lax.broadcasted_iota(jnp.int32, (8, 128), 0)
    lo4 = sub_i < 4
    lo2 = (sub_i % 4) < 2

    def regroup_rows(t):
        tu = pltpu.bitcast(t, jnp.uint32)

        def stage(a, b, sh, m):
            return jnp.where(m, a, pltpu.roll(b, sh, 0)), jnp.where(m, pltpu.roll(a, 8 - sh, 0), b)

        outs = []
        for b in range(2):
            v = [tu[hl * 16 + 8 * b: hl * 16 + 8 * b + 8, :] for hl in range(4)]
            a0, a2 = stage(v[0], v[2], 4, lo4)
            a1, a3 = stage(v[1], v[3], 4, lo4)
            b0, b1 = stage(a0, a1, 2, lo2)
            b2, b3 = stage(a2, a3, 2, lo2)
            outs += [pltpu.bitcast(z, bf16) for z in (b0, b1, b2, b3)]
        return outs

    def permute_strip(p, kt):
        blocks = regroup_rows(wqkv_v[p, pl.ds(kt * 128, 128), :].T)
        m, i = p // 8, p % 8
        for c in range(8):
            o = pl.multiple_of(m * D + c * 128 + 16 * i, 16)
            wt_v[pl.ds(o, 16), pl.ds(kt * 128, 128)] = blocks[c]

    def permute_wo(i, nt):
        blocks = regroup_rows(wo_v[_ds(i, 128), pl.ds(nt * 128, 128)])
        for c in range(8):
            o = pl.multiple_of(c * 128 + 16 * i, 16)
            wop_v[pl.ds(o, 16), pl.ds(nt * 128, 128)] = blocks[c]

    cp_x(0).start(); cp_g(0).start(); cp_u(0).start()
    for c in range(8):
        k_s[c, pl.ds(0, HALO), :] = jnp.zeros((HALO, 128), f32)
        v_s[c, pl.ds(0, HALO), :] = jnp.zeros((HALO, 128), f32)
    x_v[pl.ds(S, BM), :] = jnp.zeros((BM, D), bf16)
    cp_x(0).wait()
    cp_x(1).start()
    layernorm(0, 0, BM)
    cp_g(0).wait()
    g = _dot(xn_v[pl.ds(0, BM), :], wg_v[0])
    cp_u(0).wait()
    cp_x(2).start()
    u = _dot(xn_v[pl.ds(0, BM), :], wu_v[0])
    h_v[0, pl.ds(0, BM), pl.ds(0, FC)] = swiglu(g, u)
    cp_x(1).wait()
    layernorm(BM, 0, BM)
    cp_x(3).start(); cp_x(4).start(); cp_x(5).start()

    def g0_body(r, _):
        @pl.when(r + 5 < NRB)
        def _():
            cp_x(r + 5).start()

        @pl.when(r == 3)
        def _():
            cp_wo().start()

        @pl.when(r == 2)
        def _():
            cp_g(1).start(); cp_u(1).start()
            cp_a(0).start(); cp_a(1).start()

        @pl.when(r == 4)
        def _():
            cp_g(2).start(); cp_u(2).start()
            cp_a(2).start(); cp_a(3).start()

        @pl.when(r + 1 < NRB)
        def _():
            cp_x(r + 1).wait()

        base = pl.multiple_of(r * BM, BM)
        rows = pl.ds(base, BM)
        g = _dot(xn_v[rows, :], wg_v[0, :, pl.ds(0, 128)])
        u = _dot(xn_v[rows, :], wu_v[0, :, pl.ds(0, 128)])
        h_v[0, rows, pl.ds(0, 128)] = swiglu(g, u)
        layernorm(base, BM, LN_SPLIT)
        g = _dot(xn_v[rows, :], wg_v[0, :, pl.ds(128, 128)])
        u = _dot(xn_v[rows, :], wu_v[0, :, pl.ds(128, 128)])
        h_v[0, rows, pl.ds(128, 128)] = swiglu(g, u)
        layernorm(base, BM + LN_SPLIT, BM - LN_SPLIT)
        return 0

    lax.fori_loop(1, NRB, g0_body, 0)

    jobs = []
    for kt in range(8):
        jobs += [('a', dp, kt) for dp in range(4)] + [('o', 0, kt), ('o', 1, kt)]
    nsub = 2 * (S // BG)
    cuts = [len(jobs) * i // (nsub - 1) for i in range(nsub)] + [len(jobs)]
    NG2 = (NFC - 2) // 2

    def g_body(j, _):
        c0 = 2 * j + 1
        cp_g(c0).wait(); cp_u(c0).wait(); cp_g(c0 + 1).wait(); cp_u(c0 + 1).wait()
        for dp in range(4):
            cp_a(4 * j + dp).wait()

        @pl.when(j == 0)
        def _():
            cp_wo().wait()

        @pl.when(j + 1 < NG2)
        def _():
            cp_g(c0 + 2).start(); cp_u(c0 + 2).start(); cp_g(c0 + 3).start(); cp_u(c0 + 3).start()
            for dp in range(4):
                cp_a(4 * j + 4 + dp).start()

        @pl.when(j + 1 == NG2)
        def _():
            cp_g(NFC - 1).start(); cp_u(NFC - 1).start()

        @pl.when(j < 4)
        def _():
            cp_d(2 * j).start(); cp_d(2 * j + 1).start()

        da = jnp.minimum(j + NP, NP)
        do = pl.multiple_of(jnp.minimum(j + 64, 64) * 16, 16)
        for ib in range(nsub):
            c = c0 + ib // (S // BG)
            rows = pl.ds((ib % (S // BG)) * BG, BG)
            xn = xn_v[rows, :]
            hh = swiglu(_dot(xn, wg_v[c]), _dot(xn, wu_v[c]))
            if ib < S // BG:
                h_v[j, rows, pl.ds(FC, FC)] = hh
            else:
                h_v[j + 1, rows, pl.ds(0, FC)] = hh
            mine = jobs[cuts[ib]:cuts[ib + 1]]
            for n, (kind, dp, kt) in enumerate(mine):
                ar = (n * BG // len(mine)) // 16 * 16
                anchor = hh[ar:ar + 16, 0:128]
                if kind == 'a':
                    wqkv_v[da, 0:16, :] = anchor
                    permute_strip(4 * j + dp, kt)
                else:
                    wo_v[pl.ds(do, 16), 0:128] = anchor
                    permute_wo(jnp.minimum(2 * j + dp, 7), kt)
        return 0

    assert 4 * NG2 == NP and NG2 >= 4 and DFC == 2 * FC
    lax.fori_loop(0, NG2, g_body, 0)
    for n in range(8):
        cp_d(n).wait()
    cp_g(NFC - 1).wait(); cp_u(NFC - 1).wait()

    qscale = (DH ** -0.5) * LOG2E
    lane = lax.broadcasted_iota(jnp.int32, (TR, 128), 1)
    odd = (lane % 2) == 1
    hi2 = (lane % 4) >= 2

    def fold(x):
        y = x + jnp.where(odd, pltpu.roll(x, 1, 1), pltpu.roll(x, 127, 1))
        return y + jnp.where(hi2, pltpu.roll(y, 2, 1), pltpu.roll(y, 126, 1))

    def project(r):
        xn = xn_v[_ds(r, BM), :]
        base = pl.multiple_of(r * BM, BM) + HALO
        v = _dot(xn, wt_v[pl.ds(2 * D, D), :], NT)
        for c in range(8):
            v_s[c, pl.ds(base, BM), :] = v[:, c * 128:(c + 1) * 128]
        k = _dot(xn, wt_v[pl.ds(D, D), :], NT)
        for c in range(8):
            k_s[c, pl.ds(base, BM), :] = k[:, c * 128:(c + 1) * 128]
        q = _dot(xn, wt_v[pl.ds(0, D), :], NT) * qscale
        for c in range(8):
            q_s[c, :, :] = q[:, c * 128:(c + 1) * 128]

    def attn_qk(rb, t, chunks, st):
        acc = st.setdefault('acc', [None] * W)
        for c in chunks:
            q = q_s[c, pl.ds(t, TR), :]
            for w in range(W):
                p = q * k_s[c, pl.ds(rb + (HALO + t - DIL * w), TR), :]
                acc[w] = p if acc[w] is None else acc[w] + p

    def attn_softmax(rb, t, st):
        lg = [fold(a) for a in st.pop('acc')]
        if t < DIL * (W - 1):
            row = lax.broadcasted_iota(jnp.int32, (TR, 128), 0) + (rb + t)
            lg = [lg[0]] + [jnp.where(row >= DIL * w, lg[w], -1e9) for w in range(1, W)]
        m = lg[0]
        for w in range(1, W):
            m = jnp.maximum(m, lg[w])
        p = [jnp.exp2(l - m) for l in lg]
        den = p[0]
        for w in range(1, W):
            den = den + p[w]
        st['p'] = p
        st['rinv'] = pltpu.reciprocal(den, approx=False, full_range=False)

    def attn_pv(rb, t, chunks, st):
        p = st['p']
        for c in chunks:
            o = None
            for w in range(W):
                tt = p[w] * v_s[c, pl.ds(rb + (HALO + t - DIL * w), TR), :]
                o = tt if o is None else o + tt
            o_s[pl.ds(t, TR), pl.ds(c * 128, 128)] = (o * st['rinv']).astype(bf16)

    ntile = BM // TR
    items = []
    for t in range(ntile + 1):
        if t < ntile:
            items += [('qk', t, g) for g in range(len(QK_GROUPS))]
        if t >= 1:
            items += [('pv', t - 1, g) for g in range(len(PV_GROUPS))]
    span = NDC * SLOTS_PER - SLOT_SLACK - SLOT_FIRST
    by_slot = {}
    for i, it in enumerate(items):
        by_slot.setdefault(SLOT_FIRST + i * span // len(items), []).append(it)

    def r_body(r, _):
        rb = pl.multiple_of(r * BM, BM)
        xn = xn_v[_ds(r, BM), :]
        h_last = swiglu(_dot(xn, wg_v[NFC - 1]), _dot(xn, wu_v[NFC - 1]))
        project(r)
        dq = jnp.minimum(r + 8, 8)
        dkv = jnp.minimum(r, 7)
        sts = [dict() for _ in range(ntile)]
        acc = None
        for c in range(NDC):
            wd = jnp.concatenate([wd_v[n, pl.ds(c * DFC, DFC), :] for n in range(8)], axis=1)
            if c < NDC - 1:
                hc = h_v[c, _ds(r, BM), :]
            else:
                hc = jnp.concatenate([h_v[c, _ds(r, BM), pl.ds(0, FC)], h_last], axis=1)
            d = _dot(hc, wd)
            for u in range(SLOTS_PER):
                todo = by_slot.get(c * SLOTS_PER + u, [])
                if not todo:
                    continue
                col, row = (u // 2) * 128, (u % 2) * (BM // 2)
                anchor = d[row:row + 8, col:col + 128]
                ro = 8 * ((c * SLOTS_PER + u) % 32)
                kinds = set(k for k, _, _ in todo)
                if 'qk' in kinds:
                    q_s[dq, ro:ro + 8, :] = anchor
                    k_s[dkv, HALO + S:HALO + S + 8, :] = anchor
                if 'pv' in kinds:
                    v_s[dkv, HALO + S:HALO + S + 8, :] = anchor
                for kind, t, g in todo:
                    if kind == 'qk':
                        attn_qk(rb, t * TR, QK_GROUPS[g], sts[t])
                        if g == len(QK_GROUPS) - 1:
                            attn_softmax(rb, t * TR, sts[t])
                    else:
                        attn_pv(rb, t * TR, PV_GROUPS[g], sts[t])
            acc = d if acc is None else acc + d
        s = _dot(o_s[...], wop_v[...])
        out_v[r] = (x_v[_ds(r, BM), :].astype(f32) + s * _silu(acc)).astype(bf16)
        cp_o(r).start()
        return 0

    lax.fori_loop(0, NRB, r_body, 0)
    for r in range(NRB):
        cp_o(r).wait()


@jax.jit
def pallas_recurrent_scan__sliding_local_dilated__swiglu_ffn__prompt_kernel(
    A_x, A_wqkv, A_wo, B_x, B_w_gate, B_w_up, B_w_down,
):
    del B_x
    anyspec = pl.BlockSpec(memory_space=pl.ANY)
    out = pl.pallas_call(
        _kernel,
        out_shape=jax.ShapeDtypeStruct((S, D), bf16),
        in_specs=[anyspec] * 6,
        out_specs=anyspec,
        scratch_shapes=[
            pltpu.VMEM((S + BM, D), bf16),
            pltpu.VMEM((S + BM, D), bf16),
            pltpu.VMEM((NP + 1, D, 128), bf16),
            pltpu.VMEM((D + 64, D), bf16),
            pltpu.VMEM((NFC, D, FC), bf16),
            pltpu.VMEM((NFC, D, FC), bf16),
            pltpu.VMEM((8, F, 128), bf16),
            pltpu.VMEM((3 * D, D), bf16),
            pltpu.VMEM((D, D), bf16),
            pltpu.VMEM((NDC, S, DFC), bf16),
            pltpu.VMEM((9, BM, 128), f32),
            pltpu.VMEM((8, HALO + S + KPAD, 128), f32),
            pltpu.VMEM((8, HALO + S + KPAD, 128), f32),
            pltpu.VMEM((BM, D), bf16),
            pltpu.VMEM((NRB, BM, D), bf16),
            pltpu.SemaphoreType.DMA((NRB,)),
            pltpu.SemaphoreType.DMA((NFC,)),
            pltpu.SemaphoreType.DMA((NFC,)),
            pltpu.SemaphoreType.DMA((8,)),
            pltpu.SemaphoreType.DMA((NP + 1,)),
            pltpu.SemaphoreType.DMA((NRB,)),
        ],
        compiler_params=pltpu.CompilerParams(
            vmem_limit_bytes=120 * 1024 * 1024,
            disable_bounds_checks=True,
            disable_semaphore_checks=True,
            flags={'XLA_TPU_EVENLY_DISTRIBUTE_CRITICAL_NODES': True},
        ),
    )(A_x.reshape(S, D), A_wqkv, A_wo, B_w_gate, B_w_up, B_w_down)
    return out.reshape(1, S, D)
```
